```python
import os as _os
_os.environ.setdefault("JAX_PLATFORMS", "cpu")
import jax
import jax.numpy as jnp

def _softmax(x, axis=-1):
    return jax.nn.softmax(x, axis=axis)
def _gelu(x):
    return jax.nn.gelu(x, approximate=True)
def _silu(x):
    return jax.nn.silu(x)
def _sigmoid(x):
    return jax.nn.sigmoid(x)
def _layernorm(x, axis=-1, eps=1e-5):
    m = jnp.mean(x, axis=axis, keepdims=True)
    v = jnp.var(x, axis=axis, keepdims=True)
    return (x - m) / jnp.sqrt(v + eps)
def _scatter_add(tgt, idx, src, axis=0):
    return tgt.at[idx].add(src)
def _segment_sum(src, seg, n):
    return jax.ops.segment_sum(src, seg, n)
class _Rng:
    def __init__(self, key):
        self._k = key
    def _next(self):
        self._k, sub = jax.random.split(self._k)
        return sub
    def normal(self, shape):
        return jax.random.normal(self._next(), shape, dtype=jnp.bfloat16)
    def randint(self, lo, hi, shape):
        return jax.random.randint(self._next(), shape, lo, hi, dtype=jnp.int32)
    def uniform(self, shape, lo=0.0, hi=1.0):
        return jax.random.uniform(self._next(), shape, jnp.bfloat16, lo, hi)
    def permutation(self, n):
        return jax.random.permutation(self._next(), n)


kernel_name = 'gated_mix__softmax_full_mha__dense_activation_squared_relu__prompt'

def setup_inputs():
    _rng = _Rng(jax.random.key(int.from_bytes(__import__("os").urandom(4), "little")))
    _w = (lambda a: (lambda t: t.astype(jnp.bfloat16) if jnp.issubdtype(t.dtype, jnp.floating) else t)(jnp.asarray(a)))
    def _A_setup():
        B, S, D = 1, 2048, 640
        return {
            "x": _w((lambda *s: _rng.normal(s) * 0.05)(B, S, D)),
            "wqkv": _w((lambda *s: _rng.normal(s) * 0.4)(D, 3 * D)),
            "wo": _w((lambda *s: _rng.normal(s) * 0.05)(D, D)),
        }
    _A_in = _A_setup()

    def _B_setup():
        B, S, D, F = 1, 2048, 640, 1536
        return {
            "x": _w((lambda *s: _rng.normal(s) * 0.05)(B, S, D)),
            "w1": _w((lambda *s: _rng.normal(s) * 0.05)(D, F)),
            "b1": _w((lambda *s: _rng.normal(s) * 0.05)(F)),
            "w2": _w((lambda *s: _rng.normal(s) * 0.05)(F, D)),
            "b2": _w((lambda *s: _rng.normal(s) * 0.05)(D)),
        }
    _B_in = _B_setup()

    return {
        "A_x": _A_in["x"],
        "A_wqkv": _A_in["wqkv"],
        "A_wo": _A_in["wo"],
        "B_x": _B_in["x"],
        "B_w1": _B_in["w1"],
        "B_b1": _B_in["b1"],
        "B_w2": _B_in["w2"],
        "B_b2": _B_in["b2"],
        "gate_w": _w((lambda *s: _rng.normal(s) * 0.05)(640) * 16.0),
    }

def reference(A_x, A_wqkv, A_wo, B_x, B_w1, B_b1, B_w2, B_b2, gate_w):
    def _A_ref(x, wqkv, wo):
        B, S, D = x.shape
        H = 32; Dh = D // H
        qkv = (lambda x, *d: x.transpose(*d))((x @ wqkv).reshape(B, S, 3, H, Dh), 2, 0, 3, 1, 4)
        q, k, v = qkv[0], qkv[1], qkv[2]
        scale = Dh ** -0.5
        scores = jnp.einsum("bhqd,bhkd->bhqk", q, k) * scale
        p = _softmax(scores, axis=-1)
        o = jnp.einsum("bhqk,bhkd->bhqd", p, v)
        return (lambda x, *d: x.transpose(*d))(o, 0, 2, 1, 3).reshape(B, S, D) @ wo

    def _B_ref(x, w1, b1, w2, b2):
        h = jnp.einsum("bsd,df->bsf", x, w1) + b1
        zero = jnp.zeros_like(h)
        r = jnp.where(h > zero, h, zero)
        h = r * r
        out = jnp.einsum("bsf,fd->bsd", h, w2) + b2
        return out

    x = A_x
    g = _sigmoid((x * gate_w).sum(-1, keepdims=True))
    a = _A_ref(x, A_wqkv, A_wo)
    b = _B_ref(x, B_w1, B_b1, B_w2, B_b2)
    return g * a + (1 - g) * b
```

```python
import functools, math
import jax, jax.numpy as jnp
from jax import lax
import jax.experimental.pallas as pl
import jax.experimental.pallas.tpu as pltpu

S, D, H, DH, F = 2048, 640, 32, 20, 1536
VR = 24
NCOL = D // 128
LOG2E = 1.4426950408889634
f32, bf16, i32, i8 = jnp.float32, jnp.bfloat16, jnp.int32, jnp.int8
NN = (((1,), (0,)), ((), ()))
MAGIC = 12582912.0
QR, KR = 127.0, 254.0


def _bits(y):
    return lax.bitcast_convert_type(y, i32)


def _win(h):
    return DH * h - 4 * (h % 2)


def make(TQ=512, TK=512, NH=8, LAG=1, TA=512, TB=512, NF=1, DEP=1, force=None):
    NQ = S // TQ
    NC = S // TK
    NA = S // TA
    NB = S // TB

    def kernel(x_hbm, wqkv_hbm, wo_hbm, w1_hbm, b1_ref, w2_hbm, b2_ref, gw_ref, o_ref,
               x_sc, wqkv_sc, wo_sc, w1_sc, w2_sc, sems,
               kp_sc, qt_sc, vt_sc, kh_sc, qh_sc, bq_sc, kc_sc, ki_sc, ot_sc, yb_sc, gt_sc, flag_sc, *p_sc):
        i = pl.program_id(0)

        def x_copy(t):
            sl = pl.ds(t * TA, TA)
            return pltpu.make_async_copy(x_hbm.at[sl], x_sc.at[sl], sems.at[4 + t])

        w_copies = [pltpu.make_async_copy(s, d, sems.at[n]) for n, (s, d) in enumerate(
            [(wqkv_hbm.at[:, D:3 * D], wqkv_sc.at[:, D:3 * D]), (w1_hbm, w1_sc), (w2_hbm, w2_sc), (wo_hbm, wo_sc)])]
        wq_copy = pltpu.make_async_copy(wqkv_hbm.at[:, 0:D], wqkv_sc.at[:, 0:D], sems.at[4 + NA])

        def phase_a(t, carry):
            kmax8, vmax8 = carry
            x_copy(t).wait()
            t0 = pl.multiple_of(t * TA, TA)
            sl = pl.ds(t0, TA)
            kv = jnp.dot(x_sc[sl, :], wqkv_sc[:, D:3 * D], preferred_element_type=f32)
            k = kv[:, 0:D]
            kp_sc[sl, :] = k
            kmax8 = jnp.maximum(kmax8, jnp.max(jnp.abs(k).reshape(TA // 8, 8, D), axis=0))
            v = kv[:, D:2 * D]
            vmax8 = jnp.maximum(vmax8, jnp.max(jnp.abs(v).reshape(TA // 8, 8, D), axis=0))
            vT = v.T
            rows = lax.broadcasted_iota(i32, (8, TA), 0)
            for j in range(H // 2):
                mid = vT[40 * j + 16: 40 * j + 24]
                vt_sc[2 * j, 0:16, sl] = vT[40 * j: 40 * j + 16]
                vt_sc[2 * j, 16:24, sl] = jnp.where(rows < 4, mid, jnp.where(rows == 4, 1.0, 0.0))
                vt_sc[2 * j + 1, 0:8, sl] = jnp.where(rows >= 4, mid, jnp.where(rows == 0, 1.0, 0.0))
                vt_sc[2 * j + 1, 8:24, sl] = vT[40 * j + 24: 40 * j + 40]
            return kmax8, vmax8

        def k_split(r0, n, cols, dep):
            sl = pl.ds(r0, n)
            sw = pl.ds(pl.multiple_of(r0 // 4, n // 4), n // 4)
            for c in cols:
                inv = ki_sc[:, 128 * c:128 * (c + 1)]
                if dep is not None:
                    zero = lax.shift_right_logical(lax.shift_right_logical(_bits(dep), 31), 1)
                    inv = lax.bitcast_convert_type(_bits(inv) | zero, f32)
                kf = kp_sc[sl, 128 * c:128 * (c + 1)] * inv
                tt = kf + MAGIC
                ki = tt - MAGIC
                ta = kf * 0.5 + MAGIC
                pieces = [_bits(ta), _bits(tt) - _bits(ta), _bits((kf - ki) * 16.0 + MAGIC),
                          _bits(ki * 0.0625 + MAGIC)]
                for j, pc in enumerate(pieces):
                    w = pltpu.bitcast(pc.astype(i8), i32)
                    if j:
                        w = pltpu.roll(w, 32 * j, 1)
                    for h in range(H):
                        lo, hi = _win(h), _win(h) + 32
                        if lo // 128 == NCOL - 1 and hi > D:
                            rngs = [(lo, D), (D - 128, D - 128 + hi - D)] if c == NCOL - 1 else []
                        else:
                            a, b = max(lo, 128 * c), min(hi, 128 * (c + 1))
                            rngs = [(a, b)] if a < b else []
                        for a, b in rngs:
                            da = (a + 32 * j) % 128
                            ln = b - a
                            segs = [(da, da + ln)] if da + ln <= 128 else [(da, 128), (0, da + ln - 128)]
                            for u, v in segs:
                                kh_sc[h, sw, u:v] = w[:, u:v]

        def q_split(h, qT, sl, g2):
            rows8 = lax.broadcasted_iota(i32, (8, TB), 0)
            zpad = jnp.zeros((8, TB), i32)
            r0 = _win(h)
            qp = qT[r0:r0 + VR] * jnp.tile(kc_sc[r0:r0 + VR, :], (1, TB // 128))
            t3 = [qp[8 * e:8 * e + 8] for e in range(3)]
            if h % 2:
                t3[0] = jnp.where(rows8 >= 4, t3[0], 0.0)
            else:
                t3[2] = jnp.where(rows8 < 4, t3[2], 0.0)
            qp = jnp.concatenate(t3, axis=0)
            amax = jnp.max(jnp.abs(qp), axis=0, keepdims=True)
            g2 = jnp.maximum(g2, amax)
            am = jnp.maximum(amax, 1e-30)
            bq_sc[h, :, sl] = am * (1.0 / (QR * KR))
            rc = pl.reciprocal(am, approx=True)
            rc = rc * (2.0 - am * rc)
            qf = qp * (rc * QR)
            tt = qf + MAGIC
            qi = tt - MAGIC
            p0, p2, p3 = _bits(tt), _bits(qf * 0.0625 + MAGIC), _bits((qf - qi) * 16.0 + MAGIC)
            tiles = [zpad] * 16
            for j, pc in enumerate([p0, p0, p2, p3]):
                for e in range(3):
                    tiles[((r0 % 128) // 8 + 4 * j + e) % 16] = pc[8 * e:8 * e + 8]
            qh_sc[h, :, sl] = jnp.concatenate(tiles, axis=0).astype(i8)
            return g2

        def phase_b(t, g2):
            t0 = pl.multiple_of(t * TB, TB)
            sl = pl.ds(t0, TB)
            xt = x_sc[sl, :]
            q = jnp.dot(xt, wqkv_sc[:, 0:D], preferred_element_type=f32)
            qT = (q * (DH ** -0.5 * LOG2E)).T
            qt_sc[:, sl] = qT
            for h in range(H):
                g2 = q_split(h, qT, sl, g2)
            KB = 128
            hh = jnp.dot(xt, w1_sc[...], preferred_element_type=f32) + b1_ref[...].astype(f32).reshape(1, F)
            pcs = [(kb, c) for kb in range(TB // KB) for c in range(NCOL)]
            for n, (kb, c) in enumerate(pcs):
                pos = n * 12 * 4 // len(pcs)
                m, r = divmod(pos, 4)
                if DEP == 1:
                    dep = hh[r * (TB // 4): r * (TB // 4) + 1, 128 * m:128 * (m + 1)]
                else:
                    dep = None
                k_split(pl.multiple_of(t0 + kb * KB, KB), KB, [c], dep)
            hh = jnp.maximum(hh, 0.0)
            hh = (hh * hh).astype(bf16)
            b = jnp.dot(hh, w2_sc[...], preferred_element_type=f32) + b2_ref[...].astype(f32).reshape(1, D)
            z = jnp.sum(xt.astype(f32) * gw_ref[...].astype(f32).reshape(1, D), axis=-1, keepdims=True)
            gt = jax.nn.sigmoid(z)
            yb_sc[sl, :] = (1.0 - gt) * b
            gt_sc[sl, :] = jnp.broadcast_to(gt, (TB, 128))
            return g2

        @pl.when(i == 0)
        def _prep():
            w_copies[0].start()
            x_copy(0).start()
            w_copies[0].wait()
            for t in range(1, NA):
                x_copy(t).start()
            wq_copy.start()
            for cp in w_copies[1:]:
                cp.start()
            z8 = jnp.zeros((8, D), f32)
            kmax8, vmax8 = lax.fori_loop(0, NA, phase_a, (z8, z8))
            kmax = jnp.max(kmax8, axis=0, keepdims=True)
            ki_sc[...] = jnp.where(kmax > 0, KR / kmax, 0.0)
            for c in range(NCOL):
                kc_sc[128 * c:128 * (c + 1), :] = jnp.broadcast_to(kmax[:, 128 * c:128 * (c + 1)], (128, 128)).T
            vmax = jnp.max(vmax8)
            wq_copy.wait()
            w_copies[1].wait()
            w_copies[2].wait()
            z1 = jnp.zeros((1, TB), f32)
            g2 = lax.fori_loop(0, NB, phase_b, z1)
            amax = jnp.max(g2, axis=1, keepdims=True)
            pmax = jnp.max(jnp.exp2(jnp.minimum(amax, 4.0) * DH))
            ok = (jnp.max(amax) <= 4.0) & (vmax * pmax <= 2.0 ** 110) & (vmax * 2.0 ** 95 >= pmax)
            if force is not None:
                ok = ok & force
            flag_sc[0] = ok.astype(i32)
            flag_sc[1] = 0
            w_copies[3].wait()

        q0 = pl.multiple_of(i * TQ, TQ)

        def put_pair(h_even, oe, oo):
            rows = lax.broadcasted_iota(i32, (8, TQ), 0)
            mid = jnp.where(rows < 4, oe[16:24], oo[0:8])
            r0 = pl.multiple_of(20 * h_even, 8)
            ot_sc[pl.ds(r0, 40), :] = jnp.concatenate([oe[0:16], mid, oo[8:24]], axis=0)

        def normalize(a, odd):
            l = a[0:1, :] if odd else a[20:21, :]
            return a * (1.0 / l)

        def probs(h, qs, c, wq, bq, dst):
            kk = pltpu.bitcast(kh_sc[h, c * TK // 4:(c + 1) * TK // 4, :], i8)
            sc = lax.dot_general(kk, wq, NN, preferred_element_type=i32)
            dst[...] = pltpu.bitcast(jnp.exp2(sc.astype(f32) * bq).astype(bf16), i32)

        def fast_body(jj, carry):
            hb = jj * NH
            zz = pl.multiple_of(flag_sc[1], 8)
            outs = {}
            for u in range(NH):
                if u < NH - 1:
                    hn, qn = hb + u + 1, q0
                else:
                    last = jj == H // NH - 1
                    hn = jnp.where(last, 0, hb + NH)
                    qn = pl.multiple_of(jnp.where(last, jnp.minimum(i + 1, NQ - 1) * TQ, q0), TQ)
                wq = qh_sc[hn, :, pl.ds(qn, TQ)]
                bq = bq_sc[hn, :, pl.ds(qn, TQ)]
                acc = None
                for c in range(NC):
                    probs(hn, qn, c, wq, bq, p_sc[((u + 1) % 2) * NC + c])
                    p = pltpu.bitcast(p_sc[(u % 2) * NC + c][pl.ds(zz, TK // 2), :], bf16)
                    pv = lax.dot_general(vt_sc[hb + u, :, c * TK:(c + 1) * TK], p, NN, preferred_element_type=f32)
                    acc = pv if acc is None else pv + acc
                outs[u] = normalize(acc, u % 2)
                if u % 2 == 1:
                    put_pair(hb + u - 1, outs[u - 1], outs[u])
            return carry

        def slow_body(j, carry):
            outs = []
            SK = 256
            for u in range(2):
                h = 2 * j + u
                c0 = pl.multiple_of(jnp.minimum((DH * h) // 128, NCOL - 2) * 128, 128)
                rows = lax.broadcasted_iota(i32, (256, TQ), 0) + c0
                wq = jnp.where((rows >= DH * h) & (rows < DH * h + DH),
                               qt_sc[pl.ds(c0, 256), pl.ds(q0, TQ)], 0.0).astype(bf16)

                def chunk(c, mc):
                    m, acc = mc
                    k0 = pl.multiple_of(c * SK, SK)
                    s = lax.dot_general(kp_sc[pl.ds(k0, SK), pl.ds(c0, 256)].astype(bf16), wq, NN,
                                        preferred_element_type=f32)
                    m_new = jnp.maximum(m, jnp.max(s, axis=0, keepdims=True))
                    p = jnp.exp2(s - m_new).astype(bf16)
                    pv = lax.dot_general(vt_sc[h, :, pl.ds(k0, SK)], p, NN, preferred_element_type=f32)
                    return m_new, acc * jnp.exp2(m - m_new) + pv

                m0 = jnp.full((1, TQ), -jnp.inf, f32)
                _, acc = lax.fori_loop(0, S // SK, chunk, (m0, jnp.zeros((VR, TQ), f32)))
                outs.append(normalize(acc, u))
            put_pair(2 * j, outs[0], outs[1])
            return carry

        fast = flag_sc[0]

        @pl.when(fast == 1)
        def _():
            @pl.when(i == 0)
            def _():
                for c in range(NC):
                    probs(0, 0, c, qh_sc[0, :, 0:TQ], bq_sc[0, :, 0:TQ], p_sc[c])

            lax.fori_loop(0, H // NH, fast_body, 0)

        @pl.when(fast != 1)
        def _():
            lax.fori_loop(0, H // 2, slow_body, 0)

        o = ot_sc[...].T.astype(bf16)
        a = jnp.dot(o, wo_sc[...], preferred_element_type=f32)
        gt = jnp.tile(gt_sc[pl.ds(q0, TQ), :], (1, NCOL))
        o_ref[...] = (gt * a + yb_sc[pl.ds(q0, TQ), :]).astype(o_ref.dtype)

    def full(shape):
        return pl.BlockSpec(shape, lambda i: (0,) * len(shape))

    hbm = pl.BlockSpec(memory_space=pl.ANY)

    @jax.jit
    def fn(A_x, A_wqkv, A_wo, B_x, B_w1, B_b1, B_w2, B_b2, gate_w):
        x = A_x.reshape(S, D)
        out = pl.pallas_call(
            kernel,
            grid=(NQ,),
            in_specs=[hbm, hbm, hbm, hbm, full((F,)), hbm, full((D,)), full((D,))],
            out_specs=pl.BlockSpec((TQ, D), lambda i: (i, 0)),
            out_shape=jax.ShapeDtypeStruct((S, D), bf16),
            scratch_shapes=[
                pltpu.VMEM((S, D), bf16), pltpu.VMEM((D, 3 * D), bf16), pltpu.VMEM((D, D), bf16),
                pltpu.VMEM((D, F), bf16), pltpu.VMEM((F, D), bf16),
                pltpu.SemaphoreType.DMA((5 + NA,)),
                pltpu.VMEM((S, D), f32),
                pltpu.VMEM((D, S), f32),
                pltpu.VMEM((H, VR, S), f32),
                pltpu.VMEM((H, S // 4, 128), i32),
                pltpu.VMEM((H, 128, S), i8),
                pltpu.VMEM((H, 1, S), f32),
                pltpu.VMEM((D, 128), f32),
                pltpu.VMEM((1, D), f32),
                pltpu.VMEM((D, TQ), f32),
                pltpu.VMEM((S, D), f32),
                pltpu.VMEM((S, 128), f32),
                pltpu.SMEM((2,), i32),
            ] + [pltpu.VMEM((TK // 2, TQ), i32)] * (2 * NC),
            compiler_params=pltpu.CompilerParams(dimension_semantics=("arbitrary",),
                                                 vmem_limit_bytes=110 * 1024 * 1024),
            name=f"k8_{TQ}_{TK}_{NH}_{LAG}_{TA}_{TB}_{DEP}",
        )(x, A_wqkv, A_wo, B_w1, B_b1, B_w2, B_b2, gate_w)
        return out.reshape(1, S, D)
    return fn


_impl = make()


@jax.jit
def pallas_gated_mix__softmax_full_mha__dense_activation_squared_relu__prompt_kernel(A_x, A_wqkv, A_wo, B_x, B_w1, B_b1, B_w2, B_b2, gate_w):
    return _impl(A_x, A_wqkv, A_wo, B_x, B_w1, B_b1, B_w2, B_b2, gate_w)
```

```python
import functools, math
import jax, jax.numpy as jnp
from jax import lax
import jax.experimental.pallas as pl
import jax.experimental.pallas.tpu as pltpu

S, D, H, DH, F = 2048, 640, 32, 20, 1536
VR = 24
NCOL = D // 128
LOG2E = 1.4426950408889634
f32, bf16, i32, i8 = jnp.float32, jnp.bfloat16, jnp.int32, jnp.int8
NN = (((1,), (0,)), ((), ()))
MAGIC = 12582912.0
QR, KR = 127.0, 254.0


def _bits(y):
    return lax.bitcast_convert_type(y, i32)


def _after(v, dep):
    if dep is None:
        return v
    zero = lax.shift_right_logical(lax.shift_right_logical(_bits(dep), 31), 1)
    return lax.bitcast_convert_type(_bits(v) | zero, f32)


def _win(h):
    return DH * h - 4 * (h % 2)


def make(TQ=512, TK=512, NH=8, LAG=1, TA=512, TB=512, KB=64, M0=0, M1=4, QF=16, QS=0.3, KS=0.3, PEEL=1, STARTN=3, KV_BLOCKS=((1280, 1536), (1536, 1920), (640, 768), (768, 1280)), WAITAT=(0, 1, 1, 3), ODT=bf16, PAD0=0, PADM=0, PADE=0, ENDPAD=2, force=None):
    NQ = S // TQ
    CH = list(TK) if isinstance(TK, (tuple, list)) else [TK] * (S // TK)
    assert sum(CH) == S
    NC = len(CH)
    CO = [sum(CH[:c]) for c in range(NC + 1)]
    PSH, PKEEP = [], []
    for n, ch in enumerate(CH + CH):
        pad = PAD0 if n == 0 else PADM if n == NC else PADE
        if pad:
            PSH.append(pltpu.VMEM((1, 128 * pad), f32)); PKEEP.append(False)
        PSH.append(pltpu.VMEM((ch // 2, TQ), i32)); PKEEP.append(True)
    NA = S // TA
    NB = S // TB

    def kernel(x_hbm, wqkv_hbm, wo_hbm, w1_hbm, b1_hbm, w2_hbm, b2_hbm, gw_hbm, o_ref,
               sems, flag_sc, x_sc, wqkv_sc, wo_sc, w1_sc, w2_sc,
               kp_sc, qt_sc, vt_sc, kh_sc, qh_sc, bq_sc, ot_sc, yb_sc, gt_sc, *rest):
        p_sc = [r for r, keep in zip(rest, PKEEP) if keep]
        b1_ref, b2_ref, gw_ref, km_sc, ki_sc = rest[len(PKEEP):len(PKEEP) + 5]
        i = pl.program_id(0)

        def x_copy(t):
            sl = pl.ds(t * TA, TA)
            return pltpu.make_async_copy(x_hbm.at[sl], x_sc.at[sl], sems.at[t])

        def wcol_copy(n, lo, hi):
            return pltpu.make_async_copy(wqkv_hbm.at[:, lo:hi], wqkv_sc.at[:, lo:hi], sems.at[NA + n])

        kv_copies = [wcol_copy(n, lo, hi) for n, (lo, hi) in enumerate(KV_BLOCKS)]
        nb = len(KV_BLOCKS)
        late_copies = [wcol_copy(nb, 0, D)] + [
            pltpu.make_async_copy(s, d, sems.at[NA + nb + 1 + n]) for n, (s, d) in enumerate(
                [(w1_hbm, w1_sc), (w2_hbm, w2_sc), (b1_hbm, b1_ref), (b2_hbm, b2_ref), (gw_hbm, gw_ref), (wo_hbm, wo_sc)])]

        def phase_a(t, carry, first=False):
            kmax8, vmax8 = carry
            x_copy(t).wait()
            t0 = t * TA if first else pl.multiple_of(t * TA, TA)
            sl = pl.ds(t0, TA)
            if first:
                parts = []
                for n, (lo, hi) in enumerate(KV_BLOCKS):
                    for m in range(len(KV_BLOCKS)):
                        if WAITAT[m] == n:
                            kv_copies[m].wait()
                    if n == STARTN:
                        for tt in range(1, NA):
                            x_copy(tt).start()
                        for cp in late_copies:
                            cp.start()
                    parts.append(jnp.dot(x_sc[sl, :], wqkv_sc[:, lo:hi], preferred_element_type=f32))
                vk = jnp.concatenate(parts, axis=1)
                v, k = vk[:, 0:D], vk[:, D:2 * D]
            else:
                xt = x_sc[sl, :]
                v = jnp.dot(xt, wqkv_sc[:, 2 * D:3 * D], preferred_element_type=f32)
                k = jnp.dot(xt, wqkv_sc[:, D:2 * D], preferred_element_type=f32)
            kp_sc[sl, :] = k
            kmax8 = jnp.maximum(kmax8, jnp.max(jnp.abs(k).reshape(TA // 8, 8, D), axis=0))
            vmax8 = jnp.maximum(vmax8, jnp.max(jnp.abs(v).reshape(TA // 8, 8, D), axis=0))
            vT = v.T
            rows = lax.broadcasted_iota(i32, (8, TA), 0)
            for j in range(H // 2):
                mid = vT[40 * j + 16: 40 * j + 24]
                vt_sc[2 * j, 0:16, sl] = vT[40 * j: 40 * j + 16]
                vt_sc[2 * j, 16:24, sl] = jnp.where(rows < 4, mid, jnp.where(rows == 4, 1.0, 0.0))
                vt_sc[2 * j + 1, 0:8, sl] = jnp.where(rows >= 4, mid, jnp.where(rows == 0, 1.0, 0.0))
                vt_sc[2 * j + 1, 8:24, sl] = vT[40 * j + 24: 40 * j + 40]
            return kmax8, vmax8

        def k_split(r0, n, deps):
            sl = pl.ds(r0, n)
            sw = pl.ds(pl.multiple_of(r0 // 4, n // 4), n // 4)
            lane = lax.broadcasted_iota(i32, (n // 4, 128), 1)

            def cyc(lo, ln):
                lo %= 128
                if lo + ln <= 128:
                    return (lane >= lo) & (lane < lo + ln)
                return (lane >= lo) | (lane < lo + ln - 128)

            R = {}
            for c in range(NCOL):
                inv = ki_sc[:, 128 * c:128 * (c + 1)]
                inv = _after(inv, deps[c])
                kf = kp_sc[sl, 128 * c:128 * (c + 1)] * inv
                tt = kf + MAGIC
                ki = tt - MAGIC
                ta = kf * 0.5 + MAGIC
                pieces = [_bits(ta), _bits(tt) - _bits(ta), _bits((kf - ki) * 16.0 + MAGIC),
                          _bits(ki * 0.0625 + MAGIC)]
                Rc = []
                for j, pc in enumerate(pieces):
                    w = pltpu.bitcast(pc.astype(i8), i32)
                    Rc.append(pltpu.roll(w, 32 * j, 1) if j else w)
                R[c] = Rc
                for h in range(H):
                    ch, w0 = divmod(_win(h), 128)
                    straddle = w0 + VR > 128
                    if ch + int(straddle) != c:
                        continue
                    w = R[ch][0]
                    for j in range(4):
                        if straddle:
                            if j:
                                w = jnp.where(cyc(w0 + 32 * j, 128 - w0), R[ch][j], w)
                            w = jnp.where(cyc(32 * j, w0 + 32 - 128), R[ch + 1][j], w)
                        elif j:
                            w = jnp.where(cyc(w0 + 32 * j, 32), R[ch][j], w)
                    kh_sc[h, sw, :] = w

        def q_split(h, qT, kc, sl, g2, dep):
            rows8 = lax.broadcasted_iota(i32, (8, TB), 0)
            zpad = jnp.zeros((8, TB), i32)
            r0 = _win(h)
            qp = qT[r0:r0 + VR] * jnp.tile(_after(kc[r0:r0 + VR], dep), (1, TB // 128))
            t3 = [qp[8 * e:8 * e + 8] for e in range(3)]
            if h % 2:
                t3[0] = jnp.where(rows8 >= 4, t3[0], 0.0)
            else:
                t3[2] = jnp.where(rows8 < 4, t3[2], 0.0)
            qp = jnp.concatenate(t3, axis=0)
            amax = jnp.max(jnp.abs(qp), axis=0, keepdims=True)
            g2 = jnp.maximum(g2, amax)
            am = jnp.maximum(amax, 1e-30)
            bq_sc[h, :, sl] = am * (1.0 / (QR * KR))
            rc = pl.reciprocal(am, approx=True)
            rc = rc * (2.0 - am * rc)
            qf = qp * (rc * QR)
            tt = qf + MAGIC
            qi = tt - MAGIC
            p0, p2, p3 = _bits(tt), _bits(qf * 0.0625 + MAGIC), _bits((qf - qi) * 16.0 + MAGIC)
            tiles = [zpad] * 16
            for j, pc in enumerate([p0, p0, p2, p3]):
                for e in range(3):
                    tiles[((r0 % 128) // 8 + 4 * j + e) % 16] = pc[8 * e:8 * e + 8]
            qh_sc[h, :, sl] = jnp.concatenate(tiles, axis=0).astype(i8)
            return g2

        def phase_b(t, g2):
            t0 = pl.multiple_of(t * TB, TB)
            sl = pl.ds(t0, TB)
            xt = x_sc[sl, :]
            kc = jnp.broadcast_to(km_sc[...], (128, D)).T
            q = jnp.dot(xt, wqkv_sc[:, 0:D], preferred_element_type=f32)
            qT = (q * (DH ** -0.5 * LOG2E)).T
            qt_sc[:, sl] = qT
            hh = jnp.dot(xt, w1_sc[...], preferred_element_type=f32) + b1_ref[...].astype(f32).reshape(1, F)
            h2 = jnp.maximum(hh, 0.0)
            h2 = (h2 * h2).astype(bf16)
            b = jnp.dot(h2, w2_sc[...], preferred_element_type=f32) + b2_ref[...].astype(f32).reshape(1, D)
            pts = [(hh, m, r) for m in range(M0, 12) for r in range(8)]
            pts += [(b, m, r) for m in range(0, M1) for r in range(8) for _ in range(2)]

            def point(frac):
                arr, m, r = pts[min(int(frac * len(pts)), len(pts) - 1)]
                return arr[r * (TB // 8): r * (TB // 8) + 1, 128 * m:128 * (m + 1)]

            for h in range(H):
                g2 = q_split(h, qT, kc, sl, g2, point((h - QF + 0.5) / (H - QF) * QS) if h >= QF else None)
            npc = (TB // KB) * NCOL
            for kb in range(TB // KB):
                deps = [point(KS + (1 - KS) * (kb * NCOL + c) / npc) for c in range(NCOL)]
                k_split(pl.multiple_of(t0 + kb * KB, KB), KB, deps)
            z = jnp.sum(xt.astype(f32) * gw_ref[...].astype(f32).reshape(1, D), axis=-1, keepdims=True)
            gt = jax.nn.sigmoid(z)
            yb_sc[sl, :] = (1.0 - gt) * b
            gt_sc[sl, :] = jnp.broadcast_to(gt, (TB, 128))
            return g2

        @pl.when(i == 0)
        def _prep():
            x_copy(0).start()
            for cp in kv_copies:
                cp.start()
            z8 = jnp.zeros((8, D), f32)
            if PEEL:
                kmax8, vmax8 = lax.fori_loop(1, NA, phase_a, phase_a(0, (z8, z8), first=True))
            else:
                for cp in kv_copies:
                    cp.wait()
                for tt in range(1, NA):
                    x_copy(tt).start()
                for cp in late_copies:
                    cp.start()
                kmax8, vmax8 = lax.fori_loop(0, NA, phase_a, (z8, z8))
            kmax = jnp.max(kmax8, axis=0, keepdims=True)
            ki_sc[:, 0:D] = jnp.where(kmax > 0, KR / kmax, 0.0)
            km_sc[...] = kmax
            vmax = jnp.max(vmax8)
            for cp in late_copies:
                cp.wait()
            z1 = jnp.zeros((1, TB), f32)
            g2 = lax.fori_loop(0, NB, phase_b, z1)
            amax = jnp.max(g2, axis=1, keepdims=True)
            pmax = jnp.max(jnp.exp2(jnp.minimum(amax, 4.0) * DH))
            ok = (jnp.max(amax) <= 4.0) & (vmax * pmax <= 2.0 ** 110) & (vmax * 2.0 ** 70 >= pmax)
            if force is not None:
                ok = ok & force
            flag_sc[0] = ok.astype(i32)
            flag_sc[1] = 0

        q0 = pl.multiple_of(i * TQ, TQ)

        def put_pair(h_even, oe, oo):
            rows = lax.broadcasted_iota(i32, (8, TQ), 0)
            mid = jnp.where(rows < 4, oe[16:24], oo[0:8])
            r0 = pl.multiple_of(20 * h_even, 8)
            ot_sc[pl.ds(r0, 40), :] = jnp.concatenate([oe[0:16], mid, oo[8:24]], axis=0)

        def normalize(a, odd):
            l = a[0:1, :] if odd else a[20:21, :]
            return a * (1.0 / l)

        def probs(h, qs, c, wq, bq, dst):
            kk = pltpu.bitcast(kh_sc[h, CO[c] // 4:CO[c + 1] // 4, :], i8)
            sc = lax.dot_general(kk, wq, NN, preferred_element_type=i32)
            dst[...] = pltpu.bitcast(jnp.exp2(sc.astype(f32) * bq).astype(bf16), i32)

        def fast_body(jj, carry):
            hb = jj * NH
            zz = pl.multiple_of(flag_sc[1], 8)
            outs = {}
            for u in range(NH):
                if u < NH - 1:
                    hn, qn = hb + u + 1, q0
                else:
                    last = jj == H // NH - 1
                    hn = jnp.where(last, 0, hb + NH)
                    qn = pl.multiple_of(jnp.where(last, jnp.minimum(i + 1, NQ - 1) * TQ, q0), TQ)
                wq = qh_sc[hn, :, pl.ds(qn, TQ)]
                bq = bq_sc[hn, :, pl.ds(qn, TQ)]
                acc = None
                for c in range(NC):
                    probs(hn, qn, c, wq, bq, p_sc[((u + 1) % 2) * NC + c])
                    p = pltpu.bitcast(p_sc[(u % 2) * NC + c][pl.ds(zz, CH[c] // 2), :], bf16)
                    pv = lax.dot_general(vt_sc[hb + u, :, CO[c]:CO[c + 1]], p, NN, preferred_element_type=f32)
                    acc = pv if acc is None else pv + acc
                outs[u] = normalize(acc, u % 2)
                if u % 2 == 1:
                    put_pair(hb + u - 1, outs[u - 1], outs[u])
            return carry

        def slow_body(j, carry):
            outs = []
            SK = 256
            for u in range(2):
                h = 2 * j + u
                c0 = pl.multiple_of(jnp.minimum((DH * h) // 128, NCOL - 2) * 128, 128)
                rows = lax.broadcasted_iota(i32, (256, TQ), 0) + c0
                wq = jnp.where((rows >= DH * h) & (rows < DH * h + DH),
                               qt_sc[pl.ds(c0, 256), pl.ds(q0, TQ)], 0.0).astype(bf16)

                def chunk(c, mc):
                    m, acc = mc
                    k0 = pl.multiple_of(c * SK, SK)
                    s = lax.dot_general(kp_sc[pl.ds(k0, SK), pl.ds(c0, 256)].astype(bf16), wq, NN,
                                        preferred_element_type=f32)
                    m_new = jnp.maximum(m, jnp.max(s, axis=0, keepdims=True))
                    p = jnp.exp2(s - m_new).astype(bf16)
                    pv = lax.dot_general(vt_sc[h, :, pl.ds(k0, SK)], p, NN, preferred_element_type=f32)
                    return m_new, acc * jnp.exp2(m - m_new) + pv

                m0 = jnp.full((1, TQ), -jnp.inf, f32)
                _, acc = lax.fori_loop(0, S // SK, chunk, (m0, jnp.zeros((VR, TQ), f32)))
                outs.append(normalize(acc, u))
            put_pair(2 * j, outs[0], outs[1])
            return carry

        fast = flag_sc[0]

        @pl.when(fast == 1)
        def _():
            @pl.when(i == 0)
            def _():
                for c in range(NC):
                    probs(0, 0, c, qh_sc[0, :, 0:TQ], bq_sc[0, :, 0:TQ], p_sc[c])

            lax.fori_loop(0, H // NH, fast_body, 0)

        @pl.when(fast != 1)
        def _():
            lax.fori_loop(0, H // 2, slow_body, 0)

        o = ot_sc[...].T.astype(bf16)
        a = jnp.dot(o, wo_sc[...], preferred_element_type=f32)
        gt = jnp.tile(gt_sc[pl.ds(q0, TQ), :], (1, NCOL))
        o_ref[...] = (gt * a + yb_sc[pl.ds(q0, TQ), :]).astype(o_ref.dtype)

    def full(shape):
        return pl.BlockSpec(shape, lambda i: (0,) * len(shape))

    hbm = pl.BlockSpec(memory_space=pl.ANY)

    @jax.jit
    def fn(A_x, A_wqkv, A_wo, B_x, B_w1, B_b1, B_w2, B_b2, gate_w):
        x = A_x.reshape(S, D)
        out = pl.pallas_call(
            kernel,
            grid=(NQ,),
            in_specs=[hbm] * 8,
            out_specs=pl.BlockSpec((TQ, D), lambda i: (i, 0)),
            out_shape=jax.ShapeDtypeStruct((S, D), ODT),
            scratch_shapes=[
                pltpu.SemaphoreType.DMA((NA + len(KV_BLOCKS) + 7,)),
                pltpu.SMEM((2,), i32),
                pltpu.VMEM((S, D), bf16), pltpu.VMEM((D, 3 * D), bf16), pltpu.VMEM((D, D), bf16),
                pltpu.VMEM((D, F), bf16), pltpu.VMEM((F, D), bf16),
                pltpu.VMEM((S, D), f32),
                pltpu.VMEM((D, S), f32),
                pltpu.VMEM((H, VR, S), f32),
                pltpu.VMEM((H, S // 4, 128), i32),
                pltpu.VMEM((H, 128, S), i8),
                pltpu.VMEM((H, 1, S), f32),
                pltpu.VMEM((D, TQ), f32),
                pltpu.VMEM((S, D), f32),
                pltpu.VMEM((S, 128), f32),
            ] + PSH + [
                pltpu.VMEM((F,), bf16), pltpu.VMEM((D,), bf16), pltpu.VMEM((D,), bf16),
                pltpu.VMEM((1, D), f32), pltpu.VMEM((1, D + 128 * ENDPAD), f32),
            ],
            compiler_params=pltpu.CompilerParams(dimension_semantics=("arbitrary",),
                                                 vmem_limit_bytes=110 * 1024 * 1024),
            name=f"k15_{PAD0}_{PADM}_{PADE}_{ENDPAD}_{TQ}_{''.join(str(c // 128) for c in CH)}_{NH}_{TA}_{TB}_{KB}_{M0}_{M1}_{QF}_{int(QS*10)}_{int(KS*10)}",
        )(x, A_wqkv, A_wo, B_w1, B_b1, B_w2, B_b2, gate_w)
        return out.reshape(1, S, D)
    return fn


_impl = make(NH=16)


@jax.jit
def pallas_gated_mix__softmax_full_mha__dense_activation_squared_relu__prompt_kernel(A_x, A_wqkv, A_wo, B_x, B_w1, B_b1, B_w2, B_b2, gate_w):
    return _impl(A_x, A_wqkv, A_wo, B_x, B_w1, B_b1, B_w2, B_b2, gate_w)
```

```python
import jax
import jax.numpy as jnp
from jax import lax
import jax.experimental.pallas as pl
import jax.experimental.pallas.tpu as pltpu

S, D, H, DH, F = 2048, 640, 32, 20, 1536
VR = 24
NCOL = D // 128
TQ = 512
TK = 512
NH = 16
TT = 512
KB = 64
NQ, NC, NT = S // TQ, S // TK, S // TT
KV_BLOCKS = ((1280, 1536), (1536, 1920), (640, 768), (768, 1280))
KV_WAIT_AT = (0, 1, 1, 3)
N_LATE = 7

LOG2E = 1.4426950408889634
MAGIC = 12582912.0
QR, KR = 127.0, 254.0
AMAX_LIMIT = 4.0
TINY = 1e-30
f32, bf16, i32, i8 = jnp.float32, jnp.bfloat16, jnp.int32, jnp.int8
NN = (((1,), (0,)), ((), ()))


def _bits(y):
    return lax.bitcast_convert_type(y, i32)


def _after(v, dep):
    if dep is None:
        return v
    zero = lax.shift_right_logical(lax.shift_right_logical(_bits(dep), 31), 1)
    return lax.bitcast_convert_type(_bits(v) | zero, f32)


def _win(h):
    return DH * h - 4 * (h % 2)


def _kernel(x_hbm, wqkv_hbm, wo_hbm, w1_hbm, b1_hbm, w2_hbm, b2_hbm, gw_hbm, o_ref,
            sems, flag_sc, x_sc, wqkv_sc, wo_sc, w1_sc, w2_sc,
            kp_sc, qt_sc, vt_sc, kh_sc, qh_sc, bq_sc, ot_sc, yb_sc, gt_sc, *rest):
    p_sc = rest[:2 * NC]
    b1_sc, b2_sc, gw_sc, km_sc, ki_sc = rest[2 * NC:]
    i = pl.program_id(0)

    def x_copy(t):
        sl = pl.ds(t * TT, TT)
        return pltpu.make_async_copy(x_hbm.at[sl], x_sc.at[sl], sems.at[t])

    def wcol_copy(n, lo, hi):
        return pltpu.make_async_copy(wqkv_hbm.at[:, lo:hi], wqkv_sc.at[:, lo:hi], sems.at[NT + n])

    nkv = len(KV_BLOCKS)
    kv_copies = [wcol_copy(n, lo, hi) for n, (lo, hi) in enumerate(KV_BLOCKS)]
    late_copies = [wcol_copy(nkv, 0, D)] + [
        pltpu.make_async_copy(src, dst, sems.at[NT + nkv + 1 + n]) for n, (src, dst) in enumerate(
            [(w1_hbm, w1_sc), (w2_hbm, w2_sc), (b1_hbm, b1_sc), (b2_hbm, b2_sc), (gw_hbm, gw_sc),
             (wo_hbm, wo_sc)])]

    def phase_a(t, carry, first=False):
        kmax8, vmax8 = carry
        x_copy(t).wait()
        sl = pl.ds(t * TT if first else pl.multiple_of(t * TT, TT), TT)
        if first:
            parts = []
            for n, (lo, hi) in enumerate(KV_BLOCKS):
                for m in range(nkv):
                    if KV_WAIT_AT[m] == n:
                        kv_copies[m].wait()
                if n == nkv - 1:
                    for tt in range(1, NT):
                        x_copy(tt).start()
                    for cp in late_copies:
                        cp.start()
                parts.append(jnp.dot(x_sc[sl, :], wqkv_sc[:, lo:hi], preferred_element_type=f32))
            vk = jnp.concatenate(parts, axis=1)
            v, k = vk[:, 0:D], vk[:, D:2 * D]
        else:
            xt = x_sc[sl, :]
            v = jnp.dot(xt, wqkv_sc[:, 2 * D:3 * D], preferred_element_type=f32)
            k = jnp.dot(xt, wqkv_sc[:, D:2 * D], preferred_element_type=f32)
        kp_sc[sl, :] = k
        kmax8 = jnp.maximum(kmax8, jnp.max(jnp.abs(k).reshape(TT // 8, 8, D), axis=0))
        vmax8 = jnp.maximum(vmax8, jnp.max(jnp.abs(v).reshape(TT // 8, 8, D), axis=0))
        vT = v.T
        rows = lax.broadcasted_iota(i32, (8, TT), 0)
        for j in range(H // 2):
            mid = vT[40 * j + 16:40 * j + 24]
            vt_sc[2 * j, 0:16, sl] = vT[40 * j:40 * j + 16]
            vt_sc[2 * j, 16:24, sl] = jnp.where(rows < 4, mid, jnp.where(rows == 4, 1.0, 0.0))
            vt_sc[2 * j + 1, 0:8, sl] = jnp.where(rows >= 4, mid, jnp.where(rows == 0, 1.0, 0.0))
            vt_sc[2 * j + 1, 8:24, sl] = vT[40 * j + 24:40 * j + 40]
        return kmax8, vmax8

    def k_split(r0, deps):
        sl = pl.ds(r0, KB)
        sw = pl.ds(pl.multiple_of(r0 // 4, KB // 4), KB // 4)
        lane = lax.broadcasted_iota(i32, (KB // 4, 128), 1)

        def cyc(lo, n):
            lo %= 128
            if lo + n <= 128:
                return (lane >= lo) & (lane < lo + n)
            return (lane >= lo) | (lane < lo + n - 128)

        limbs = {}
        for c in range(NCOL):
            cs = slice(128 * c, 128 * (c + 1))
            kf = kp_sc[sl, cs] * _after(ki_sc[:, cs], deps[c])
            tk = kf + MAGIC
            ki = tk - MAGIC
            ta = kf * 0.5 + MAGIC
            raw = [_bits(ta), _bits(tk) - _bits(ta), _bits((kf - ki) * 16.0 + MAGIC),
                   _bits(ki * 0.0625 + MAGIC)]
            words = [pltpu.bitcast(r.astype(i8), i32) for r in raw]
            limbs[c] = [pltpu.roll(w, 32 * j, 1) if j else w for j, w in enumerate(words)]
            for h in range(H):
                ch, w0 = divmod(_win(h), 128)
                straddle = w0 + VR > 128
                if ch + int(straddle) != c:
                    continue
                w = limbs[ch][0]
                for j in range(4):
                    if straddle:
                        if j:
                            w = jnp.where(cyc(w0 + 32 * j, 128 - w0), limbs[ch][j], w)
                        w = jnp.where(cyc(32 * j, w0 + 32 - 128), limbs[ch + 1][j], w)
                    elif j:
                        w = jnp.where(cyc(w0 + 32 * j, 32), limbs[ch][j], w)
                kh_sc[h, sw, :] = w

    def q_split(h, qT, kcol, sl, dep):
        rows = lax.broadcasted_iota(i32, (8, TT), 0)
        r0 = _win(h)
        qp = qT[r0:r0 + VR] * jnp.tile(_after(kcol[r0:r0 + VR], dep), (1, TT // 128))
        t3 = [qp[8 * e:8 * e + 8] for e in range(3)]
        if h % 2:
            t3[0] = jnp.where(rows >= 4, t3[0], 0.0)
        else:
            t3[2] = jnp.where(rows < 4, t3[2], 0.0)
        qp = jnp.concatenate(t3, axis=0)
        amax = jnp.maximum(jnp.max(jnp.abs(qp), axis=0, keepdims=True), TINY)
        bq_sc[h, :, sl] = amax * (1.0 / (QR * KR))
        rc = pl.reciprocal(amax, approx=True)
        rc = rc * (2.0 - amax * rc)
        qf = qp * (rc * QR)
        tq = qf + MAGIC
        qi = tq - MAGIC
        raw = [_bits(tq), _bits(tq), _bits(qf * 0.0625 + MAGIC), _bits((qf - qi) * 16.0 + MAGIC)]
        tiles = [jnp.zeros((8, TT), i32)] * 16
        for j, r in enumerate(raw):
            for e in range(3):
                tiles[((r0 % 128) // 8 + 4 * j + e) % 16] = r[8 * e:8 * e + 8]
        qh_sc[h, :, sl] = jnp.concatenate(tiles, axis=0).astype(i8)
        return amax

    def phase_b(t, amax):
        t0 = pl.multiple_of(t * TT, TT)
        sl = pl.ds(t0, TT)
        xt = x_sc[sl, :]
        kcol = jnp.broadcast_to(km_sc[...], (128, D)).T
        q = jnp.dot(xt, wqkv_sc[:, 0:D], preferred_element_type=f32)
        qT = (q * (DH ** -0.5 * LOG2E)).T
        qt_sc[:, sl] = qT
        hh = jnp.dot(xt, w1_sc[...], preferred_element_type=f32) + b1_sc[...].astype(f32).reshape(1, F)
        h2 = jnp.maximum(hh, 0.0)
        h2 = (h2 * h2).astype(bf16)
        b = jnp.dot(h2, w2_sc[...], preferred_element_type=f32) + b2_sc[...].astype(f32).reshape(1, D)

        pts = [(hh, m, r) for m in range(F // 128) for r in range(8)]
        pts += [(b, m, r) for m in range(NCOL - 1) for r in range(8) for _ in range(2)]

        def point(frac):
            arr, m, r = pts[min(int(frac * len(pts)), len(pts) - 1)]
            return arr[r * (TT // 8):r * (TT // 8) + 1, 128 * m:128 * (m + 1)]

        for h in range(H):
            dep = point(0.3 * (h - H // 2 + 0.5) / (H // 2)) if h >= H // 2 else None
            amax = jnp.maximum(amax, q_split(h, qT, kcol, sl, dep))
        npc = (TT // KB) * NCOL
        for kb in range(TT // KB):
            k_split(pl.multiple_of(t0 + kb * KB, KB),
                    [point(0.3 + 0.7 * (kb * NCOL + c) / npc) for c in range(NCOL)])

        z = jnp.sum(xt.astype(f32) * gw_sc[...].astype(f32).reshape(1, D), axis=-1, keepdims=True)
        g = jax.nn.sigmoid(z)
        yb_sc[sl, :] = (1.0 - g) * b
        gt_sc[sl, :] = jnp.broadcast_to(g, (TT, 128))
        return amax

    @pl.when(i == 0)
    def _prepare():
        x_copy(0).start()
        for cp in kv_copies:
            cp.start()
        z8 = jnp.zeros((8, D), f32)
        kmax8, vmax8 = lax.fori_loop(1, NT, phase_a, phase_a(0, (z8, z8), first=True))
        kmax = jnp.maximum(jnp.max(kmax8, axis=0, keepdims=True), TINY)
        km_sc[...] = kmax
        ki_sc[:, 0:D] = KR / kmax
        vmax = jnp.max(vmax8)
        for cp in late_copies:
            cp.wait()
        amax = lax.fori_loop(0, NT, phase_b, jnp.zeros((1, TT), f32))
        amax = jnp.max(amax, axis=1, keepdims=True)
        pmax = jnp.max(jnp.exp2(jnp.minimum(amax, AMAX_LIMIT) * DH))
        safe = (jnp.max(amax) <= AMAX_LIMIT) & (vmax * pmax <= 2.0 ** 110) & (vmax * 2.0 ** 70 >= pmax)
        flag_sc[0] = safe.astype(i32)
        flag_sc[1] = 0

    q0 = pl.multiple_of(i * TQ, TQ)

    def normalize(acc, odd):
        return acc * (1.0 / (acc[0:1, :] if odd else acc[DH:DH + 1, :]))

    def put_pair(h_even, oe, oo):
        rows = lax.broadcasted_iota(i32, (8, TQ), 0)
        mid = jnp.where(rows < 4, oe[16:24], oo[0:8])
        ot_sc[pl.ds(pl.multiple_of(DH * h_even, 8), 2 * DH), :] = jnp.concatenate(
            [oe[0:16], mid, oo[8:24]], axis=0)

    def probs(h, c, wq, bq, dst):
        kk = pltpu.bitcast(kh_sc[h, c * TK // 4:(c + 1) * TK // 4, :], i8)
        sc = lax.dot_general(kk, wq, NN, preferred_element_type=i32)
        dst[...] = pltpu.bitcast(jnp.exp2(sc.astype(f32) * bq).astype(bf16), i32)

    def fast_body(jj, carry):
        hb = jj * NH
        zz = pl.multiple_of(flag_sc[1], 8)
        outs = []
        for u in range(NH):
            if u < NH - 1:
                hn, qn = hb + u + 1, q0
            else:
                last = jj == H // NH - 1
                hn = jnp.where(last, 0, hb + NH)
                qn = pl.multiple_of(jnp.where(last, jnp.minimum(i + 1, NQ - 1) * TQ, q0), TQ)
            wq = qh_sc[hn, :, pl.ds(qn, TQ)]
            bq = bq_sc[hn, :, pl.ds(qn, TQ)]
            acc = None
            for c in range(NC):
                probs(hn, c, wq, bq, p_sc[((u + 1) % 2) * NC + c])
                p = pltpu.bitcast(p_sc[(u % 2) * NC + c][pl.ds(zz, TK // 2), :], bf16)
                pv = lax.dot_general(vt_sc[hb + u, :, c * TK:(c + 1) * TK], p, NN,
                                     preferred_element_type=f32)
                acc = pv if acc is None else pv + acc
            outs.append(normalize(acc, u % 2))
            if u % 2:
                put_pair(hb + u - 1, outs[u - 1], outs[u])
        return carry

    def exact_max_body(j, carry):
        sk = 256
        outs = []
        for u in range(2):
            h = 2 * j + u
            c0 = pl.multiple_of(jnp.minimum((DH * h) // 128, NCOL - 2) * 128, 128)
            rows = lax.broadcasted_iota(i32, (256, TQ), 0) + c0
            wq = jnp.where((rows >= DH * h) & (rows < DH * h + DH),
                           qt_sc[pl.ds(c0, 256), pl.ds(q0, TQ)], 0.0).astype(bf16)

            def chunk(c, mc, h=h, c0=c0, wq=wq):
                m, acc = mc
                k0 = pl.multiple_of(c * sk, sk)
                s = lax.dot_general(kp_sc[pl.ds(k0, sk), pl.ds(c0, 256)].astype(bf16), wq, NN,
                                    preferred_element_type=f32)
                m_new = jnp.maximum(m, jnp.max(s, axis=0, keepdims=True))
                p = jnp.exp2(s - m_new).astype(bf16)
                pv = lax.dot_general(vt_sc[h, :, pl.ds(k0, sk)], p, NN, preferred_element_type=f32)
                return m_new, acc * jnp.exp2(m - m_new) + pv

            init = (jnp.full((1, TQ), -jnp.inf, f32), jnp.zeros((VR, TQ), f32))
            outs.append(normalize(lax.fori_loop(0, S // sk, chunk, init)[1], u))
        put_pair(2 * j, outs[0], outs[1])
        return carry

    safe = flag_sc[0]

    @pl.when(safe == 1)
    def _():
        @pl.when(i == 0)
        def _():
            for c in range(NC):
                probs(0, c, qh_sc[0, :, 0:TQ], bq_sc[0, :, 0:TQ], p_sc[c])

        lax.fori_loop(0, H // NH, fast_body, 0)

    @pl.when(safe != 1)
    def _():
        lax.fori_loop(0, H // 2, exact_max_body, 0)

    a = jnp.dot(ot_sc[...].T.astype(bf16), wo_sc[...], preferred_element_type=f32)
    g = jnp.tile(gt_sc[pl.ds(q0, TQ), :], (1, NCOL))
    o_ref[...] = (g * a + yb_sc[pl.ds(q0, TQ), :]).astype(o_ref.dtype)


@jax.jit
def pallas_gated_mix__softmax_full_mha__dense_activation_squared_relu__prompt_kernel(
    A_x: jax.Array,
    A_wqkv: jax.Array,
    A_wo: jax.Array,
    B_x: jax.Array,
    B_w1: jax.Array,
    B_b1: jax.Array,
    B_w2: jax.Array,
    B_b2: jax.Array,
    gate_w: jax.Array,
):
    del B_x
    vmem = pltpu.VMEM
    scratch = [
        pltpu.SemaphoreType.DMA((NT + len(KV_BLOCKS) + N_LATE,)),
        pltpu.SMEM((2,), i32),
        vmem((S, D), bf16), vmem((D, 3 * D), bf16), vmem((D, D), bf16),
        vmem((D, F), bf16), vmem((F, D), bf16),
        vmem((S, D), f32),
        vmem((D, S), f32),
        vmem((H, VR, S), f32),
        vmem((H, S // 4, 128), i32),
        vmem((H, 128, S), i8),
        vmem((H, 1, S), f32),
        vmem((D, TQ), f32),
        vmem((S, D), f32),
        vmem((S, 128), f32),
    ] + [vmem((TK // 2, TQ), i32)] * (2 * NC) + [
        vmem((F,), bf16), vmem((D,), bf16), vmem((D,), bf16),
        vmem((1, D), f32), vmem((1, D + 256), f32),
    ]
    out = pl.pallas_call(
        _kernel,
        grid=(NQ,),
        in_specs=[pl.BlockSpec(memory_space=pl.ANY)] * 8,
        out_specs=pl.BlockSpec((TQ, D), lambda i: (i, 0)),
        out_shape=jax.ShapeDtypeStruct((S, D), bf16),
        scratch_shapes=scratch,
        compiler_params=pltpu.CompilerParams(dimension_semantics=("arbitrary",),
                                             vmem_limit_bytes=100 * 1024 * 1024),
        name="gated_mix_mha_ffn",
    )(A_x.reshape(S, D), A_wqkv, A_wo, B_w1, B_b1, B_w2, B_b2, gate_w)
    return out.reshape(1, S, D)
```

```python
import jax
import jax.numpy as jnp
from jax import lax
import jax.experimental.pallas as pl
import jax.experimental.pallas.tpu as pltpu

S, D, H, DH, F = 2048, 640, 32, 20, 1536
VR = 24
NCOL = D // 128
TQ = 512
TK = 512
NH = 16
TT = 512
KB = 64
NQ, NC, NT = S // TQ, S // TK, S // TT
KV_BLOCKS = ((1280, 1536), (1536, 1920), (640, 768), (768, 1280))
KV_WAIT_AT = (0, 1, 1, 3)
N_LATE = 7

LOG2E = 1.4426950408889634
MAGIC = 12582912.0
QR, KR = 127.0, 254.0
AMAX_LIMIT = 4.0
TINY = 1e-30
f32, bf16, i32, i8 = jnp.float32, jnp.bfloat16, jnp.int32, jnp.int8
NN = (((1,), (0,)), ((), ()))


def _bits(y):
    return lax.bitcast_convert_type(y, i32)


def _after(v, dep):
    if dep is None:
        return v
    zero = lax.shift_right_logical(lax.shift_right_logical(_bits(dep), 31), 1)
    return lax.bitcast_convert_type(_bits(v) | zero, f32)


def _win(h):
    return DH * h - 4 * (h % 2)


def _kernel(x_hbm, wqkv_hbm, wo_hbm, w1_hbm, b1_hbm, w2_hbm, b2_hbm, gw_hbm, o_ref,
            sems, flag_sc, x_sc, wqkv_sc, wo_sc, w1_sc, w2_sc,
            kp_sc, qt_sc, vt_sc, kh_sc, qh_sc, bq_sc, ot_sc, yb_sc, gt_sc, *rest):
    p_sc = rest[:2 * NC]
    b1_sc, b2_sc, gw_sc, km_sc, ki_sc = rest[2 * NC:]
    i = pl.program_id(0)

    def x_copy(t):
        sl = pl.ds(t * TT, TT)
        return pltpu.make_async_copy(x_hbm.at[sl], x_sc.at[sl], sems.at[t])

    def wcol_copy(n, lo, hi):
        return pltpu.make_async_copy(wqkv_hbm.at[:, lo:hi], wqkv_sc.at[:, lo:hi], sems.at[NT + n])

    nkv = len(KV_BLOCKS)
    kv_copies = [wcol_copy(n, lo, hi) for n, (lo, hi) in enumerate(KV_BLOCKS)]
    late_copies = [wcol_copy(nkv, 0, D)] + [
        pltpu.make_async_copy(src, dst, sems.at[NT + nkv + 1 + n]) for n, (src, dst) in enumerate(
            [(w1_hbm, w1_sc), (w2_hbm, w2_sc), (b1_hbm, b1_sc), (b2_hbm, b2_sc), (gw_hbm, gw_sc),
             (wo_hbm, wo_sc)])]

    def phase_a(t, carry, first=False):
        kmax8, vmax8 = carry
        x_copy(t).wait()
        sl = pl.ds(t * TT if first else pl.multiple_of(t * TT, TT), TT)
        if first:
            parts = []
            for n, (lo, hi) in enumerate(KV_BLOCKS):
                for m in range(nkv):
                    if KV_WAIT_AT[m] == n:
                        kv_copies[m].wait()
                if n == nkv - 1:
                    for tt in range(1, NT):
                        x_copy(tt).start()
                    for cp in late_copies:
                        cp.start()
                parts.append(jnp.dot(x_sc[sl, :], wqkv_sc[:, lo:hi], preferred_element_type=f32))
            vk = jnp.concatenate(parts, axis=1)
            v, k = vk[:, 0:D], vk[:, D:2 * D]
        else:
            xt = x_sc[sl, :]
            v = jnp.dot(xt, wqkv_sc[:, 2 * D:3 * D], preferred_element_type=f32)
            k = jnp.dot(xt, wqkv_sc[:, D:2 * D], preferred_element_type=f32)
        kp_sc[sl, :] = k
        kmax8 = jnp.maximum(kmax8, jnp.max(jnp.abs(k).reshape(TT // 8, 8, D), axis=0))
        vmax8 = jnp.maximum(vmax8, jnp.max(jnp.abs(v).reshape(TT // 8, 8, D), axis=0))
        vT = v.T
        rows = lax.broadcasted_iota(i32, (8, TT), 0)
        for j in range(H // 2):
            mid = vT[40 * j + 16:40 * j + 24]
            vt_sc[2 * j, 0:16, sl] = vT[40 * j:40 * j + 16]
            vt_sc[2 * j, 16:24, sl] = jnp.where(rows < 4, mid, jnp.where(rows == 4, 1.0, 0.0))
            vt_sc[2 * j + 1, 0:8, sl] = jnp.where(rows >= 4, mid, jnp.where(rows == 0, 1.0, 0.0))
            vt_sc[2 * j + 1, 8:24, sl] = vT[40 * j + 24:40 * j + 40]
        return kmax8, vmax8

    def k_split(r0, deps):
        sl = pl.ds(r0, KB)
        sw = pl.ds(pl.multiple_of(r0 // 4, KB // 4), KB // 4)
        lane = lax.broadcasted_iota(i32, (KB // 4, 128), 1)

        def cyc(lo, n):
            lo %= 128
            if lo + n <= 128:
                return (lane >= lo) & (lane < lo + n)
            return (lane >= lo) | (lane < lo + n - 128)

        limbs = {}
        for c in range(NCOL):
            cs = slice(128 * c, 128 * (c + 1))
            kf = kp_sc[sl, cs] * _after(ki_sc[:, cs], deps[c])
            tk = kf + MAGIC
            ki = tk - MAGIC
            ta = kf * 0.5 + MAGIC
            raw = [_bits(ta), _bits(tk) - _bits(ta), _bits((kf - ki) * 16.0 + MAGIC),
                   _bits(ki * 0.0625 + MAGIC)]
            words = [pltpu.bitcast(r.astype(i8), i32) for r in raw]
            limbs[c] = [pltpu.roll(w, 32 * j, 1) if j else w for j, w in enumerate(words)]
            for h in range(H):
                ch, w0 = divmod(_win(h), 128)
                straddle = w0 + VR > 128
                if ch + int(straddle) != c:
                    continue
                w = limbs[ch][0]
                for j in range(4):
                    if straddle:
                        if j:
                            w = jnp.where(cyc(w0 + 32 * j, 128 - w0), limbs[ch][j], w)
                        w = jnp.where(cyc(32 * j, w0 + 32 - 128), limbs[ch + 1][j], w)
                    elif j:
                        w = jnp.where(cyc(w0 + 32 * j, 32), limbs[ch][j], w)
                kh_sc[h, sw, :] = w

    def q_split(h, qT, kcol, sl, dep):
        rows = lax.broadcasted_iota(i32, (8, TT), 0)
        r0 = _win(h)
        qp = qT[r0:r0 + VR] * jnp.tile(_after(kcol[r0:r0 + VR], dep), (1, TT // 128))
        t3 = [qp[8 * e:8 * e + 8] for e in range(3)]
        if h % 2:
            t3[0] = jnp.where(rows >= 4, t3[0], 0.0)
        else:
            t3[2] = jnp.where(rows < 4, t3[2], 0.0)
        qp = jnp.concatenate(t3, axis=0)
        amax = jnp.maximum(jnp.max(jnp.abs(qp), axis=0, keepdims=True), TINY)
        bq_sc[h, :, sl] = amax * (1.0 / (QR * KR))
        rc = pl.reciprocal(amax, approx=True)
        rc = rc * (2.0 - amax * rc)
        qf = qp * (rc * QR)
        tq = qf + MAGIC
        qi = tq - MAGIC
        raw = [_bits(tq), _bits(tq), _bits(qf * 0.0625 + MAGIC), _bits((qf - qi) * 16.0 + MAGIC)]
        tiles = [jnp.zeros((8, TT), i32)] * 16
        for j, r in enumerate(raw):
            for e in range(3):
                tiles[((r0 % 128) // 8 + 4 * j + e) % 16] = r[8 * e:8 * e + 8]
        qh_sc[h, :, sl] = jnp.concatenate(tiles, axis=0).astype(i8)
        return amax

    def phase_b(t, amax):
        t0 = pl.multiple_of(t * TT, TT)
        sl = pl.ds(t0, TT)
        xt = x_sc[sl, :]
        kcol = jnp.broadcast_to(km_sc[...], (128, D)).T
        q = jnp.dot(xt, wqkv_sc[:, 0:D], preferred_element_type=f32)
        qT = (q * (DH ** -0.5 * LOG2E)).T
        qt_sc[:, sl] = qT
        hh = jnp.dot(xt, w1_sc[...], preferred_element_type=f32) + b1_sc[...].astype(f32).reshape(1, F)
        h2 = jnp.maximum(hh, 0.0)
        h2 = (h2 * h2).astype(bf16)
        b = jnp.dot(h2, w2_sc[...], preferred_element_type=f32) + b2_sc[...].astype(f32).reshape(1, D)

        pts = [(hh, m, r) for m in range(F // 128) for r in range(8)]
        pts += [(b, m, r) for m in range(NCOL - 1) for r in range(8) for _ in range(2)]

        def point(frac):
            arr, m, r = pts[min(int(frac * len(pts)), len(pts) - 1)]
            return arr[r * (TT // 8):r * (TT // 8) + 1, 128 * m:128 * (m + 1)]

        for h in range(H):
            dep = point(0.3 * (h - H // 2 + 0.5) / (H // 2)) if h >= H // 2 else None
            amax = jnp.maximum(amax, q_split(h, qT, kcol, sl, dep))
        npc = (TT // KB) * NCOL
        for kb in range(TT // KB):
            k_split(pl.multiple_of(t0 + kb * KB, KB),
                    [point(0.3 + 0.7 * (kb * NCOL + c) / npc) for c in range(NCOL)])

        z = jnp.sum(xt.astype(f32) * gw_sc[...].astype(f32).reshape(1, D), axis=-1, keepdims=True)
        g = jax.nn.sigmoid(z)
        yb_sc[sl, :] = (1.0 - g) * b
        gt_sc[sl, :] = jnp.broadcast_to(g, (TT, 128))
        return amax

    def probs(h, c, wq, bq, dst):
        kk = pltpu.bitcast(kh_sc[h, c * TK // 4:(c + 1) * TK // 4, :], i8)
        sc = lax.dot_general(kk, wq, NN, preferred_element_type=i32)
        dst[...] = pltpu.bitcast(jnp.exp2(sc.astype(f32) * bq).astype(bf16), i32)

    @pl.when(i == 0)
    def _prepare():
        x_copy(0).start()
        for cp in kv_copies:
            cp.start()
        z8 = jnp.zeros((8, D), f32)
        kmax8, vmax8 = lax.fori_loop(1, NT, phase_a, phase_a(0, (z8, z8), first=True))
        kmax = jnp.maximum(jnp.max(kmax8, axis=0, keepdims=True), TINY)
        km_sc[...] = kmax
        ki_sc[:, 0:D] = KR / kmax
        vmax = jnp.max(vmax8)
        for cp in late_copies:
            cp.wait()
        amax = lax.fori_loop(0, NT, phase_b, jnp.zeros((1, TT), f32))
        amax = jnp.max(amax, axis=1, keepdims=True)
        pmax = jnp.max(jnp.exp2(jnp.minimum(amax, AMAX_LIMIT) * DH))
        safe = (jnp.max(amax) <= AMAX_LIMIT) & (vmax * pmax <= 2.0 ** 110) & (vmax * 2.0 ** 70 >= pmax)
        flag_sc[0] = safe.astype(i32)
        for c in range(NC):
            probs(0, c, qh_sc[0, :, 0:TQ], bq_sc[0, :, 0:TQ], p_sc[c])

    q0 = pl.multiple_of(i * TQ, TQ)

    def normalize(acc, odd):
        return acc * (1.0 / (acc[0:1, :] if odd else acc[DH:DH + 1, :]))

    def put_pair(h_even, oe, oo):
        rows = lax.broadcasted_iota(i32, (8, TQ), 0)
        mid = jnp.where(rows < 4, oe[16:24], oo[0:8])
        ot_sc[pl.ds(pl.multiple_of(DH * h_even, 8), 2 * DH), :] = jnp.concatenate(
            [oe[0:16], mid, oo[8:24]], axis=0)

    def fast_body(jj, carry):
        hb = jj * NH
        zz = pl.multiple_of(lax.shift_right_logical(jj, 16) * 8, 8)
        outs = []
        for u in range(NH):
            if u < NH - 1:
                hn, qn = hb + u + 1, q0
            else:
                last = jj == H // NH - 1
                hn = jnp.where(last, 0, hb + NH)
                qn = pl.multiple_of(jnp.where(last, jnp.minimum(i + 1, NQ - 1) * TQ, q0), TQ)
            wq = qh_sc[hn, :, pl.ds(qn, TQ)]
            bq = bq_sc[hn, :, pl.ds(qn, TQ)]
            acc = None
            for c in range(NC):
                probs(hn, c, wq, bq, p_sc[((u + 1) % 2) * NC + c])
                p = pltpu.bitcast(p_sc[(u % 2) * NC + c][pl.ds(zz, TK // 2), :], bf16)
                pv = lax.dot_general(vt_sc[hb + u, :, c * TK:(c + 1) * TK], p, NN,
                                     preferred_element_type=f32)
                acc = pv if acc is None else pv + acc
            outs.append(normalize(acc, u % 2))
            if u % 2:
                put_pair(hb + u - 1, outs[u - 1], outs[u])
        return carry

    def exact_max_body(j, carry):
        sk = 256
        outs = []
        for u in range(2):
            h = 2 * j + u
            c0 = pl.multiple_of(jnp.minimum((DH * h) // 128, NCOL - 2) * 128, 128)
            rows = lax.broadcasted_iota(i32, (256, TQ), 0) + c0
            wq = jnp.where((rows >= DH * h) & (rows < DH * h + DH),
                           qt_sc[pl.ds(c0, 256), pl.ds(q0, TQ)], 0.0).astype(bf16)

            def chunk(c, mc, h=h, c0=c0, wq=wq):
                m, acc = mc
                k0 = pl.multiple_of(c * sk, sk)
                s = lax.dot_general(kp_sc[pl.ds(k0, sk), pl.ds(c0, 256)].astype(bf16), wq, NN,
                                    preferred_element_type=f32)
                m_new = jnp.maximum(m, jnp.max(s, axis=0, keepdims=True))
                p = jnp.exp2(s - m_new).astype(bf16)
                pv = lax.dot_general(vt_sc[h, :, pl.ds(k0, sk)], p, NN, preferred_element_type=f32)
                return m_new, acc * jnp.exp2(m - m_new) + pv

            init = (jnp.full((1, TQ), -jnp.inf, f32), jnp.zeros((VR, TQ), f32))
            outs.append(normalize(lax.fori_loop(0, S // sk, chunk, init)[1], u))
        put_pair(2 * j, outs[0], outs[1])
        return carry

    lax.cond(flag_sc[0] == 1,
             lambda: lax.fori_loop(0, H // NH, fast_body, 0),
             lambda: lax.fori_loop(0, H // 2, exact_max_body, 0))

    a = jnp.dot(ot_sc[...].T.astype(bf16), wo_sc[...], preferred_element_type=f32)
    g = jnp.tile(gt_sc[pl.ds(q0, TQ), :], (1, NCOL))
    o_ref[...] = (g * a + yb_sc[pl.ds(q0, TQ), :]).astype(o_ref.dtype)


@jax.jit
def pallas_gated_mix__softmax_full_mha__dense_activation_squared_relu__prompt_kernel(
    A_x: jax.Array,
    A_wqkv: jax.Array,
    A_wo: jax.Array,
    B_x: jax.Array,
    B_w1: jax.Array,
    B_b1: jax.Array,
    B_w2: jax.Array,
    B_b2: jax.Array,
    gate_w: jax.Array,
):
    del B_x
    vmem = pltpu.VMEM
    scratch = [
        pltpu.SemaphoreType.DMA((NT + len(KV_BLOCKS) + N_LATE,)),
        pltpu.SMEM((1,), i32),
        vmem((S, D), bf16), vmem((D, 3 * D), bf16), vmem((D, D), bf16),
        vmem((D, F), bf16), vmem((F, D), bf16),
        vmem((S, D), f32),
        vmem((D, S), f32),
        vmem((H, VR, S), f32),
        vmem((H, S // 4, 128), i32),
        vmem((H, 128, S), i8),
        vmem((H, 1, S), f32),
        vmem((D, TQ), f32),
        vmem((S, D), f32),
        vmem((S, 128), f32),
    ] + [vmem((TK // 2, TQ), i32)] * (2 * NC) + [
        vmem((F,), bf16), vmem((D,), bf16), vmem((D,), bf16),
        vmem((1, D), f32), vmem((1, D + 256), f32),
    ]
    out = pl.pallas_call(
        _kernel,
        grid=(NQ,),
        in_specs=[pl.BlockSpec(memory_space=pl.ANY)] * 8,
        out_specs=pl.BlockSpec((TQ, D), lambda i: (i, 0)),
        out_shape=jax.ShapeDtypeStruct((S, D), bf16),
        scratch_shapes=scratch,
        compiler_params=pltpu.CompilerParams(dimension_semantics=("arbitrary",),
                                             vmem_limit_bytes=100 * 1024 * 1024),
        name="gated_mix_mha_ffn",
    )(A_x.reshape(S, D), A_wqkv, A_wo, B_w1, B_b1, B_w2, B_b2, gate_w)
    return out.reshape(1, S, D)
```

```python
import jax
import jax.numpy as jnp
from jax import lax
import jax.experimental.pallas as pl
import jax.experimental.pallas.tpu as pltpu

S, D, H, DH, F = 2048, 640, 32, 20, 1536
VR = 24
NCOL = D // 128
TQ = 512
TK = 512
NH = 16
TT = 512
KB = 64
NQ, NC, NT = S // TQ, S // TK, S // TT
KV_BLOCKS = ((1280, 1536), (1536, 1920), (640, 768), (768, 1280))
KV_WAIT_AT = (0, 1, 1, 3)
N_LATE = 7
NO = 4

LOG2E = 1.4426950408889634
MAGIC = 12582912.0
QR, KR = 127.0, 254.0
AMAX_LIMIT = 4.0
TINY = 1e-30
f32, bf16, i32, i8 = jnp.float32, jnp.bfloat16, jnp.int32, jnp.int8
NN = (((1,), (0,)), ((), ()))


def _bits(y):
    return lax.bitcast_convert_type(y, i32)


def _zero_after(dep_bits):
    return lax.shift_right_logical(lax.shift_right_logical(dep_bits, 31), 1)


def _after(v, dep):
    if dep is None:
        return v
    return lax.bitcast_convert_type(_bits(v) | _zero_after(_bits(dep)), f32)


def _win(h):
    return DH * h - 4 * (h % 2)


def _kernel(x_hbm, wqkv_hbm, wo_hbm, w1_hbm, b1_hbm, w2_hbm, b2_hbm, gw_hbm, o_hbm,
            sems, osems, flag_sc, os_sc, wot_sc, x_sc, wqkv_sc, wo_sc, w1_sc, w2_sc,
            kp_sc, qt_sc, vt_sc, kh_sc, qh_sc, bq_sc, ot_sc, yb_sc, gt_sc, *rest):
    p_sc = rest[:2 * NC]
    b1_sc, b2_sc, gw_sc, km_sc, ki_sc = rest[2 * NC:]
    i = pl.program_id(0)

    def x_copy(t):
        sl = pl.ds(t * TT, TT)
        return pltpu.make_async_copy(x_hbm.at[sl], x_sc.at[sl], sems.at[t])

    def wcol_copy(n, lo, hi):
        return pltpu.make_async_copy(wqkv_hbm.at[:, lo:hi], wqkv_sc.at[:, lo:hi], sems.at[NT + n])

    nkv = len(KV_BLOCKS)
    kv_copies = [wcol_copy(n, lo, hi) for n, (lo, hi) in enumerate(KV_BLOCKS)]
    late_copies = [wcol_copy(nkv, 0, D)] + [
        pltpu.make_async_copy(src, dst, sems.at[NT + nkv + 1 + n]) for n, (src, dst) in enumerate(
            [(w1_hbm, w1_sc), (w2_hbm, w2_sc), (b1_hbm, b1_sc), (b2_hbm, b2_sc), (gw_hbm, gw_sc),
             (wo_hbm, wo_sc)])]

    def phase_a(t, carry, first=False):
        kmax8, vmax8 = carry
        x_copy(t).wait()
        sl = pl.ds(t * TT if first else pl.multiple_of(t * TT, TT), TT)
        if first:
            parts = []
            for n, (lo, hi) in enumerate(KV_BLOCKS):
                for m in range(nkv):
                    if KV_WAIT_AT[m] == n:
                        kv_copies[m].wait()
                if n == nkv - 1:
                    for tt in range(1, NT):
                        x_copy(tt).start()
                    for cp in late_copies:
                        cp.start()
                parts.append(jnp.dot(x_sc[sl, :], wqkv_sc[:, lo:hi], preferred_element_type=f32))
            vk = jnp.concatenate(parts, axis=1)
            v, k = vk[:, 0:D], vk[:, D:2 * D]
        else:
            xt = x_sc[sl, :]
            v = jnp.dot(xt, wqkv_sc[:, 2 * D:3 * D], preferred_element_type=f32)
            k = jnp.dot(xt, wqkv_sc[:, D:2 * D], preferred_element_type=f32)
        kp_sc[sl, :] = k
        kmax8 = jnp.maximum(kmax8, jnp.max(jnp.abs(k).reshape(TT // 8, 8, D), axis=0))
        vmax8 = jnp.maximum(vmax8, jnp.max(jnp.abs(v).reshape(TT // 8, 8, D), axis=0))
        vT = v.T
        rows = lax.broadcasted_iota(i32, (8, TT), 0)
        for j in range(H // 2):
            mid = vT[40 * j + 16:40 * j + 24]
            vt_sc[2 * j, 0:16, sl] = vT[40 * j:40 * j + 16]
            vt_sc[2 * j, 16:24, sl] = jnp.where(rows < 4, mid, jnp.where(rows == 4, 1.0, 0.0))
            vt_sc[2 * j + 1, 0:8, sl] = jnp.where(rows >= 4, mid, jnp.where(rows == 0, 1.0, 0.0))
            vt_sc[2 * j + 1, 8:24, sl] = vT[40 * j + 24:40 * j + 40]
        return kmax8, vmax8

    def k_split(r0, deps):
        sl = pl.ds(r0, KB)
        sw = pl.ds(pl.multiple_of(r0 // 4, KB // 4), KB // 4)
        lane = lax.broadcasted_iota(i32, (KB // 4, 128), 1)

        def cyc(lo, n):
            lo %= 128
            if lo + n <= 128:
                return (lane >= lo) & (lane < lo + n)
            return (lane >= lo) | (lane < lo + n - 128)

        limbs = {}
        for c in range(NCOL):
            cs = slice(128 * c, 128 * (c + 1))
            kf = kp_sc[sl, cs] * _after(ki_sc[:, cs], deps[c])
            tk = kf + MAGIC
            ki = tk - MAGIC
            ta = kf * 0.5 + MAGIC
            raw = [_bits(ta), _bits(tk) - _bits(ta), _bits((kf - ki) * 16.0 + MAGIC),
                   _bits(ki * 0.0625 + MAGIC)]
            words = [pltpu.bitcast(r.astype(i8), i32) for r in raw]
            limbs[c] = [pltpu.roll(w, 32 * j, 1) if j else w for j, w in enumerate(words)]
            for h in range(H):
                ch, w0 = divmod(_win(h), 128)
                straddle = w0 + VR > 128
                if ch + int(straddle) != c:
                    continue
                w = limbs[ch][0]
                for j in range(4):
                    if straddle:
                        if j:
                            w = jnp.where(cyc(w0 + 32 * j, 128 - w0), limbs[ch][j], w)
                        w = jnp.where(cyc(32 * j, w0 + 32 - 128), limbs[ch + 1][j], w)
                    elif j:
                        w = jnp.where(cyc(w0 + 32 * j, 32), limbs[ch][j], w)
                kh_sc[h, sw, :] = w

    def q_split(h, qT, kcol, sl, dep):
        rows = lax.broadcasted_iota(i32, (8, TT), 0)
        r0 = _win(h)
        qp = qT[r0:r0 + VR] * jnp.tile(_after(kcol[r0:r0 + VR], dep), (1, TT // 128))
        t3 = [qp[8 * e:8 * e + 8] for e in range(3)]
        if h % 2:
            t3[0] = jnp.where(rows >= 4, t3[0], 0.0)
        else:
            t3[2] = jnp.where(rows < 4, t3[2], 0.0)
        qp = jnp.concatenate(t3, axis=0)
        amax = jnp.maximum(jnp.max(jnp.abs(qp), axis=0, keepdims=True), TINY)
        bq_sc[h, :, sl] = amax * (1.0 / (QR * KR))
        rc = pl.reciprocal(amax, approx=True)
        rc = rc * (2.0 - amax * rc)
        qf = qp * (rc * QR)
        tq = qf + MAGIC
        qi = tq - MAGIC
        raw = [_bits(tq), _bits(tq), _bits(qf * 0.0625 + MAGIC), _bits((qf - qi) * 16.0 + MAGIC)]
        tiles = [jnp.zeros((8, TT), i32)] * 16
        for j, r in enumerate(raw):
            for e in range(3):
                tiles[((r0 % 128) // 8 + 4 * j + e) % 16] = r[8 * e:8 * e + 8]
        qh_sc[h, :, sl] = jnp.concatenate(tiles, axis=0).astype(i8)
        return amax

    def phase_b(t, amax):
        t0 = pl.multiple_of(t * TT, TT)
        sl = pl.ds(t0, TT)
        xt = x_sc[sl, :]
        kcol = jnp.broadcast_to(km_sc[...], (128, D)).T
        q = jnp.dot(xt, wqkv_sc[:, 0:D], preferred_element_type=f32)
        qT = (q * (DH ** -0.5 * LOG2E)).T
        qt_sc[:, sl] = qT
        hh = jnp.dot(xt, w1_sc[...], preferred_element_type=f32) + b1_sc[...].astype(f32).reshape(1, F)
        h2 = jnp.maximum(hh, 0.0)
        h2 = (h2 * h2).astype(bf16)
        b = jnp.dot(h2, w2_sc[...], preferred_element_type=f32) + b2_sc[...].astype(f32).reshape(1, D)

        pts = [(hh, m, r) for m in range(F // 128) for r in range(8)]
        pts += [(b, m, r) for m in range(NCOL - 1) for r in range(8) for _ in range(2)]

        def point(frac):
            arr, m, r = pts[min(int(frac * len(pts)), len(pts) - 1)]
            return arr[r * (TT // 8):r * (TT // 8) + 1, 128 * m:128 * (m + 1)]

        for h in range(H):
            dep = point(0.3 * (h - H // 2 + 0.5) / (H // 2)) if h >= H // 2 else None
            amax = jnp.maximum(amax, q_split(h, qT, kcol, sl, dep))
        npc = (TT // KB) * NCOL
        for kb in range(TT // KB):
            k_split(pl.multiple_of(t0 + kb * KB, KB),
                    [point(0.3 + 0.7 * (kb * NCOL + c) / npc) for c in range(NCOL)])

        z = jnp.sum(xt.astype(f32) * gw_sc[...].astype(f32).reshape(1, D), axis=-1, keepdims=True)
        g = jax.nn.sigmoid(z)
        yb_sc[sl, :] = (1.0 - g) * b
        gt_sc[sl, :] = jnp.broadcast_to(g, (TT, 128))
        return amax

    def probs(h, c, wq, bq, dst):
        kk = pltpu.bitcast(kh_sc[h, c * TK // 4:(c + 1) * TK // 4, :], i8)
        sc = lax.dot_general(kk, wq, NN, preferred_element_type=i32)
        dst[...] = pltpu.bitcast(jnp.exp2(sc.astype(f32) * bq).astype(bf16), i32)
        return sc[0:8]

    @pl.when(i == 0)
    def _prepare():
        x_copy(0).start()
        for cp in kv_copies:
            cp.start()
        z8 = jnp.zeros((8, D), f32)
        kmax8, vmax8 = lax.fori_loop(1, NT, phase_a, phase_a(0, (z8, z8), first=True))
        kmax = jnp.maximum(jnp.max(kmax8, axis=0, keepdims=True), TINY)
        km_sc[...] = kmax
        ki_sc[:, 0:D] = KR / kmax
        vmax = jnp.max(vmax8)
        for cp in late_copies:
            cp.wait()
        amax = lax.fori_loop(0, NT, phase_b, jnp.zeros((1, TT), f32))
        amax = jnp.max(amax, axis=1, keepdims=True)
        pmax = jnp.max(jnp.exp2(jnp.minimum(amax, AMAX_LIMIT) * DH))
        safe = (jnp.max(amax) <= AMAX_LIMIT) & (vmax * pmax <= 2.0 ** 110) & (vmax * 2.0 ** 70 >= pmax)
        flag_sc[0] = safe.astype(i32)
        wot_sc[...] = wo_sc[...].astype(f32).T.astype(bf16)
        for c in range(NC):
            probs(0, c, qh_sc[0, :, 0:TQ], bq_sc[0, :, 0:TQ], p_sc[c])

    q0 = pl.multiple_of(i * TQ, TQ)

    def normalize(acc, odd):
        return acc * (1.0 / (acc[0:1, :] if odd else acc[DH:DH + 1, :]))

    def put_pair(h_even, oe, oo):
        rows = lax.broadcasted_iota(i32, (8, TQ), 0)
        mid = jnp.where(rows < 4, oe[16:24], oo[0:8])
        ot_sc[pl.ds(pl.multiple_of(DH * h_even, 8), 2 * DH), :] = jnp.concatenate(
            [oe[0:16], mid, oo[8:24]], axis=0)

    def fast_body(jj, carry):
        hb = jj * NH
        zz = pl.multiple_of(lax.shift_right_logical(jj, 16) * 8, 8)
        outs = []
        for u in range(NH):
            if u < NH - 1:
                hn, qn = hb + u + 1, q0
            else:
                last = jj == H // NH - 1
                hn = jnp.where(last, 0, hb + NH)
                qn = pl.multiple_of(jnp.where(last, jnp.minimum(i + 1, NQ - 1) * TQ, q0), TQ)
            wq = qh_sc[hn, :, pl.ds(qn, TQ)]
            bq = bq_sc[hn, :, pl.ds(qn, TQ)]
            acc = None
            for c in range(NC):
                zero = _zero_after(probs(hn, c, wq, bq, p_sc[((u + 1) % 2) * NC + c]))
                pw = p_sc[(u % 2) * NC + c][pl.ds(zz, TK // 2), :]
                pw = jnp.concatenate([piece for e in range(0, TK // 2, 64)
                                      for piece in (pw[e:e + 56], pw[e + 56:e + 64] | zero)], axis=0)
                p = pltpu.bitcast(pw, bf16)
                pv = lax.dot_general(vt_sc[hb + u, :, c * TK:(c + 1) * TK], p, NN,
                                     preferred_element_type=f32)
                acc = pv if acc is None else pv + acc
            outs.append(normalize(acc, u % 2))
            if u % 2:
                put_pair(hb + u - 1, outs[u - 1], outs[u])
        return carry

    def exact_max_body(j, carry):
        sk = 256
        outs = []
        for u in range(2):
            h = 2 * j + u
            c0 = pl.multiple_of(jnp.minimum((DH * h) // 128, NCOL - 2) * 128, 128)
            rows = lax.broadcasted_iota(i32, (256, TQ), 0) + c0
            wq = jnp.where((rows >= DH * h) & (rows < DH * h + DH),
                           qt_sc[pl.ds(c0, 256), pl.ds(q0, TQ)], 0.0).astype(bf16)

            def chunk(c, mc, h=h, c0=c0, wq=wq):
                m, acc = mc
                k0 = pl.multiple_of(c * sk, sk)
                s = lax.dot_general(kp_sc[pl.ds(k0, sk), pl.ds(c0, 256)].astype(bf16), wq, NN,
                                    preferred_element_type=f32)
                m_new = jnp.maximum(m, jnp.max(s, axis=0, keepdims=True))
                p = jnp.exp2(s - m_new).astype(bf16)
                pv = lax.dot_general(vt_sc[h, :, pl.ds(k0, sk)], p, NN, preferred_element_type=f32)
                return m_new, acc * jnp.exp2(m - m_new) + pv

            init = (jnp.full((1, TQ), -jnp.inf, f32), jnp.zeros((VR, TQ), f32))
            outs.append(normalize(lax.fori_loop(0, S // sk, chunk, init)[1], u))
        put_pair(2 * j, outs[0], outs[1])
        return carry

    lax.cond(flag_sc[0] == 1,
             lambda: lax.fori_loop(0, H // NH, fast_body, 0),
             lambda: lax.fori_loop(0, H // 2, exact_max_body, 0))

    def out_copy(step, n):
        r = n * (TQ // NO)
        return pltpu.make_async_copy(os_sc.at[pl.ds(r, TQ // NO)], o_hbm.at[pl.ds(step * TQ + r, TQ // NO)],
                                     osems.at[n])

    @pl.when(i > 0)
    def _():
        for n in range(NO):
            out_copy(i - 1, n).wait()

    for n in range(NO):
        r, m = n * (TQ // NO), TQ // NO
        if n == 0:
            a = jnp.dot(wot_sc[...], ot_sc[:, r:r + m].astype(bf16), preferred_element_type=f32).T
        else:
            a = jnp.dot(ot_sc[:, r:r + m].T.astype(bf16), wo_sc[...], preferred_element_type=f32)
        rs = pl.ds(pl.multiple_of(q0 + r, m), m)
        g = jnp.tile(gt_sc[rs, :], (1, NCOL))
        os_sc[r:r + m, :] = (g * a + yb_sc[rs, :]).astype(bf16)
        out_copy(i, n).start()

    @pl.when(i == NQ - 1)
    def _():
        for n in range(NO):
            out_copy(i, n).wait()


@jax.jit
def pallas_gated_mix__softmax_full_mha__dense_activation_squared_relu__prompt_kernel(
    A_x: jax.Array,
    A_wqkv: jax.Array,
    A_wo: jax.Array,
    B_x: jax.Array,
    B_w1: jax.Array,
    B_b1: jax.Array,
    B_w2: jax.Array,
    B_b2: jax.Array,
    gate_w: jax.Array,
):
    del B_x
    vmem = pltpu.VMEM
    scratch = [
        pltpu.SemaphoreType.DMA((NT + len(KV_BLOCKS) + N_LATE,)),
        pltpu.SemaphoreType.DMA((NO,)),
        pltpu.SMEM((1,), i32),
        vmem((TQ, D), bf16),
        vmem((D, D), bf16),
        vmem((S, D), bf16), vmem((D, 3 * D), bf16), vmem((D, D), bf16),
        vmem((D, F), bf16), vmem((F, D), bf16),
        vmem((S, D), f32),
        vmem((D, S), f32),
        vmem((H, VR, S), f32),
        vmem((H, S // 4, 128), i32),
        vmem((H, 128, S), i8),
        vmem((H, 1, S), f32),
        vmem((D, TQ), f32),
        vmem((S, D), f32),
        vmem((S, 128), f32),
    ] + [vmem((TK // 2, TQ), i32)] * (2 * NC) + [
        vmem((F,), bf16), vmem((D,), bf16), vmem((D,), bf16),
        vmem((1, D), f32), vmem((1, D + 256), f32),
    ]
    out = pl.pallas_call(
        _kernel,
        grid=(NQ,),
        in_specs=[pl.BlockSpec(memory_space=pl.ANY)] * 8,
        out_specs=pl.BlockSpec(memory_space=pl.ANY),
        out_shape=jax.ShapeDtypeStruct((S, D), bf16),
        scratch_shapes=scratch,
        compiler_params=pltpu.CompilerParams(dimension_semantics=("arbitrary",),
                                             vmem_limit_bytes=100 * 1024 * 1024),
        name="gated_mix_mha_ffn",
    )(A_x.reshape(S, D), A_wqkv, A_wo, B_w1, B_b1, B_w2, B_b2, gate_w)
    return out.reshape(1, S, D)
```

```python
import jax
import jax.numpy as jnp
from jax import lax
import jax.experimental.pallas as pl
import jax.experimental.pallas.tpu as pltpu

S, D, H, DH, F = 2048, 640, 32, 20, 1536
VR = 24
NCOL = D // 128
TQ = 512
TK = 512
NH = 16
TT = 512
KB = 32
NQ, NC, NT = S // TQ, S // TK, S // TT
KV_BLOCKS = ((1280, 1536), (1536, 1920), (640, 768), (768, 1280))
KV_WAIT_AT = (0, 1, 1, 3)
N_LATE = 7
NO = 4

LOG2E = 1.4426950408889634
SCALE_BF16 = 0.2236328125
MAGIC = 12582912.0
QR, KR = 127.0, 254.0
AMAX_LIMIT = 4.0
TINY = 1e-30
f32, bf16, i32, i8 = jnp.float32, jnp.bfloat16, jnp.int32, jnp.int8
NN = (((1,), (0,)), ((), ()))


def _bits(y):
    return lax.bitcast_convert_type(y, i32)


def _zero_after(dep_bits):
    return lax.shift_right_logical(lax.shift_right_logical(dep_bits, 31), 1)


def _after(v, dep):
    if dep is None:
        return v
    return lax.bitcast_convert_type(_bits(v) | _zero_after(_bits(dep)), f32)


def _win(h):
    return DH * h - 4 * (h % 2)


def _kernel(x_hbm, wqkv_hbm, wo_hbm, w1_hbm, b1_hbm, w2_hbm, b2_hbm, gw_hbm, o_hbm,
            sems, osems, flag_sc, os_sc, wot_sc, x_sc, wqkv_sc, wo_sc, w1_sc, w2_sc,
            kp_sc, qt_sc, vt_sc, kh_sc, qh_sc, bq_sc, ot_sc, yb_sc, gt_sc, *rest):
    p_sc = rest[:2 * NC]
    b1_sc, b2_sc, gw_sc, km_sc, ki_sc = rest[2 * NC:]
    i = pl.program_id(0)

    def x_copy(t):
        sl = pl.ds(t * TT, TT)
        return pltpu.make_async_copy(x_hbm.at[sl], x_sc.at[sl], sems.at[t])

    def wcol_copy(n, lo, hi):
        return pltpu.make_async_copy(wqkv_hbm.at[:, lo:hi], wqkv_sc.at[:, lo:hi], sems.at[NT + n])

    nkv = len(KV_BLOCKS)
    kv_copies = [wcol_copy(n, lo, hi) for n, (lo, hi) in enumerate(KV_BLOCKS)]
    late_copies = [wcol_copy(nkv, 0, D)] + [
        pltpu.make_async_copy(src, dst, sems.at[NT + nkv + 1 + n]) for n, (src, dst) in enumerate(
            [(w1_hbm, w1_sc), (w2_hbm, w2_sc), (b1_hbm, b1_sc), (b2_hbm, b2_sc), (gw_hbm, gw_sc),
             (wo_hbm, wo_sc)])]

    def phase_a(t, carry, first=False):
        kmax8, vmax8 = carry
        x_copy(t).wait()
        sl = pl.ds(t * TT if first else pl.multiple_of(t * TT, TT), TT)
        if first:
            parts = []
            for n, (lo, hi) in enumerate(KV_BLOCKS):
                for m in range(nkv):
                    if KV_WAIT_AT[m] == n:
                        kv_copies[m].wait()
                if n == nkv - 1:
                    for tt in range(1, NT):
                        x_copy(tt).start()
                    for cp in late_copies:
                        cp.start()
                parts.append(jnp.dot(x_sc[sl, :], wqkv_sc[:, lo:hi], preferred_element_type=f32))
            vk = jnp.concatenate(parts, axis=1)
            v, k = vk[:, 0:D], vk[:, D:2 * D]
        else:
            xt = x_sc[sl, :]
            v = jnp.dot(xt, wqkv_sc[:, 2 * D:3 * D], preferred_element_type=f32)
            k = jnp.dot(xt, wqkv_sc[:, D:2 * D], preferred_element_type=f32)
        kp_sc[sl, :] = k
        kmax8 = jnp.maximum(kmax8, jnp.max(jnp.abs(k).reshape(TT // 8, 8, D), axis=0))
        vmax8 = jnp.maximum(vmax8, jnp.max(jnp.abs(v).reshape(TT // 8, 8, D), axis=0))
        vT = v.T
        rows = lax.broadcasted_iota(i32, (8, TT), 0)
        for j in range(H // 2):
            mid = vT[40 * j + 16:40 * j + 24]
            vt_sc[2 * j, 0:16, sl] = vT[40 * j:40 * j + 16]
            vt_sc[2 * j, 16:24, sl] = jnp.where(rows < 4, mid, jnp.where(rows == 4, 1.0, 0.0))
            vt_sc[2 * j + 1, 0:8, sl] = jnp.where(rows >= 4, mid, jnp.where(rows == 0, 1.0, 0.0))
            vt_sc[2 * j + 1, 8:24, sl] = vT[40 * j + 24:40 * j + 40]
        return kmax8, vmax8

    def k_split(r0, deps):
        sl = pl.ds(r0, KB)
        sw = pl.ds(pl.multiple_of(r0 // 4, KB // 4), KB // 4)
        lane = lax.broadcasted_iota(i32, (KB // 4, 128), 1)

        def cyc(lo, n):
            lo %= 128
            if lo + n <= 128:
                return (lane >= lo) & (lane < lo + n)
            return (lane >= lo) | (lane < lo + n - 128)

        limbs = {}
        for c in range(NCOL):
            cs = slice(128 * c, 128 * (c + 1))
            kf = kp_sc[sl, cs] * _after(ki_sc[:, cs], deps[c])
            tk = kf + MAGIC
            ki = tk - MAGIC
            ta = kf * 0.5 + MAGIC
            raw = [_bits(ta), _bits(tk) - _bits(ta), _bits((kf - ki) * 16.0 + MAGIC),
                   _bits(ki * 0.0625 + MAGIC)]
            words = [pltpu.bitcast(r.astype(i8), i32) for r in raw]
            limbs[c] = [pltpu.roll(w, 32 * j, 1) if j else w for j, w in enumerate(words)]
            for h in range(H):
                ch, w0 = divmod(_win(h), 128)
                straddle = w0 + VR > 128
                if ch + int(straddle) != c:
                    continue
                w = limbs[ch][0]
                for j in range(4):
                    if straddle:
                        if j:
                            w = jnp.where(cyc(w0 + 32 * j, 128 - w0), limbs[ch][j], w)
                        w = jnp.where(cyc(32 * j, w0 + 32 - 128), limbs[ch + 1][j], w)
                    elif j:
                        w = jnp.where(cyc(w0 + 32 * j, 32), limbs[ch][j], w)
                kh_sc[h, sw, :] = w

    def q_split(h, qT, kcol, sl, dep):
        rows = lax.broadcasted_iota(i32, (8, TT), 0)
        r0 = _win(h)
        qp = qT[r0:r0 + VR] * jnp.tile(_after(kcol[r0:r0 + VR], dep), (1, TT // 128))
        t3 = [qp[8 * e:8 * e + 8] for e in range(3)]
        if h % 2:
            t3[0] = jnp.where(rows >= 4, t3[0], 0.0)
        else:
            t3[2] = jnp.where(rows < 4, t3[2], 0.0)
        qp = jnp.concatenate(t3, axis=0)
        amax = jnp.maximum(jnp.max(jnp.abs(qp), axis=0, keepdims=True), TINY)
        bq_sc[h, :, sl] = amax * (1.0 / (QR * KR))
        rc = pl.reciprocal(amax, approx=True)
        rc = rc * (2.0 - amax * rc)
        qf = qp * (rc * QR)
        tq = qf + MAGIC
        qi = tq - MAGIC
        raw = [_bits(tq), _bits(tq), _bits(qf * 0.0625 + MAGIC), _bits((qf - qi) * 16.0 + MAGIC)]
        tiles = [jnp.zeros((8, TT), i32)] * 16
        for j, r in enumerate(raw):
            for e in range(3):
                tiles[((r0 % 128) // 8 + 4 * j + e) % 16] = r[8 * e:8 * e + 8]
        qh_sc[h, :, sl] = jnp.concatenate(tiles, axis=0).astype(i8)
        return amax

    def phase_b(t, amax):
        t0 = pl.multiple_of(t * TT, TT)
        sl = pl.ds(t0, TT)
        xt = x_sc[sl, :]
        kcol = jnp.broadcast_to(km_sc[...], (128, D)).T
        q = jnp.dot(xt, wqkv_sc[:, 0:D], preferred_element_type=f32)
        qT = (q * 0.25).T
        qt_sc[:, sl] = qT
        hh = jnp.dot(xt, w1_sc[...], preferred_element_type=f32) + b1_sc[...].astype(f32).reshape(1, F)
        h2 = jnp.maximum(hh, 0.0)
        h2 = (h2 * h2).astype(bf16)
        hb = TT // 2
        bs = [jnp.dot(h2[e * hb:(e + 1) * hb], w2_sc[...], preferred_element_type=f32) for e in range(2)]
        b = jnp.concatenate(bs, axis=0) + b2_sc[...].astype(f32).reshape(1, D)

        pts = [(hh, m, r) for m in range(F // 128) for r in range(8)]
        pts += [(b, m, 4 * e + r) for e in range(2) for m in range(NCOL - e) for r in range(4) for _ in range(2)]

        def point(frac):
            arr, m, r = pts[min(int(frac * len(pts)), len(pts) - 1)]
            return arr[r * (TT // 8):r * (TT // 8) + 1, 128 * m:128 * (m + 1)]

        for h in range(H):
            dep = point(0.3 * (h - H // 2 + 0.5) / (H // 2)) if h >= H // 2 else None
            amax = jnp.maximum(amax, q_split(h, qT, kcol, sl, dep))
        npc = (TT // KB) * NCOL
        for kb in range(TT // KB):
            k_split(pl.multiple_of(t0 + kb * KB, KB),
                    [point(0.3 + 0.7 * (kb * NCOL + c) / npc) for c in range(NCOL)])

        z = jnp.sum(xt.astype(f32) * gw_sc[...].astype(f32).reshape(1, D), axis=-1, keepdims=True)
        g = jax.nn.sigmoid(z)
        yb_sc[sl, :] = (1.0 - g) * b
        gt_sc[sl, :] = jnp.broadcast_to(g, (TT, 128))
        return amax

    def probs(h, c, wq, bq, dst):
        kk = pltpu.bitcast(kh_sc[h, c * TK // 4:(c + 1) * TK // 4, :], i8)
        sc = lax.dot_general(kk, wq, NN, preferred_element_type=i32)
        dst[...] = pltpu.bitcast(jnp.exp2(sc.astype(f32) * bq).astype(bf16), i32)
        return sc[0:8]

    @pl.when(i == 0)
    def _prepare():
        x_copy(0).start()
        for cp in kv_copies:
            cp.start()
        z8 = jnp.zeros((8, D), f32)
        kmax8, vmax8 = lax.fori_loop(1, NT, phase_a, phase_a(0, (z8, z8), first=True))
        kmax = jnp.maximum(jnp.max(kmax8, axis=0, keepdims=True), TINY)
        km_sc[...] = kmax * (4.0 * DH ** -0.5 * LOG2E)
        ki_sc[:, 0:D] = KR / kmax
        vmax = jnp.max(vmax8)
        for cp in late_copies:
            cp.wait()
        amax = lax.fori_loop(0, NT, phase_b, jnp.zeros((1, TT), f32))
        amax = jnp.max(amax, axis=1, keepdims=True)
        pmax = jnp.max(jnp.exp2(jnp.minimum(amax, AMAX_LIMIT) * DH))
        safe = (jnp.max(amax) <= AMAX_LIMIT) & (vmax * pmax <= 2.0 ** 110) & (vmax * 2.0 ** 70 >= pmax)
        flag_sc[0] = safe.astype(i32)
        wot_sc[...] = wo_sc[...].astype(f32).T
        for c in range(NC):
            probs(0, c, qh_sc[0, :, 0:TQ], bq_sc[0, :, 0:TQ], p_sc[c])

    q0 = pl.multiple_of(i * TQ, TQ)

    def normalize(acc, odd):
        return acc * (1.0 / (acc[0:1, :] if odd else acc[DH:DH + 1, :]))

    def put_pair(h_even, oe, oo):
        rows = lax.broadcasted_iota(i32, (8, TQ), 0)
        mid = jnp.where(rows < 4, oe[16:24], oo[0:8])
        ot_sc[pl.ds(pl.multiple_of(DH * h_even, 8), 2 * DH), :] = jnp.concatenate(
            [oe[0:16], mid, oo[8:24]], axis=0)

    def fast_body(jj, carry):
        hb = jj * NH
        zz = pl.multiple_of(lax.shift_right_logical(jj, 16) * 8, 8)
        outs = []
        for u in range(NH):
            if u < NH - 1:
                hn, qn = hb + u + 1, q0
            else:
                last = jj == H // NH - 1
                hn = jnp.where(last, 0, hb + NH)
                qn = pl.multiple_of(jnp.where(last, jnp.minimum(i + 1, NQ - 1) * TQ, q0), TQ)
            wq = qh_sc[hn, :, pl.ds(qn, TQ)]
            bq = bq_sc[hn, :, pl.ds(qn, TQ)]
            acc = None
            for c in range(NC):
                zero = _zero_after(probs(hn, c, wq, bq, p_sc[((u + 1) % 2) * NC + c]))
                pw = p_sc[(u % 2) * NC + c][pl.ds(zz, TK // 2), :]
                pw = jnp.concatenate([piece for e in range(0, TK // 2, 64)
                                      for piece in (pw[e:e + 56], pw[e + 56:e + 64] | zero)], axis=0)
                p = pltpu.bitcast(pw, bf16)
                pv = lax.dot_general(vt_sc[hb + u, :, c * TK:(c + 1) * TK], p, NN,
                                     preferred_element_type=f32)
                acc = pv if acc is None else pv + acc
            outs.append(normalize(acc, u % 2))
            if u % 2:
                put_pair(hb + u - 1, outs[u - 1], outs[u])
        return carry

    def exact_max_body(j, carry):
        sk = 256
        outs = []
        for u in range(2):
            h = 2 * j + u
            c0 = pl.multiple_of(jnp.minimum((DH * h) // 128, NCOL - 2) * 128, 128)
            rows = lax.broadcasted_iota(i32, (256, TQ), 0) + c0
            wq = jnp.where((rows >= DH * h) & (rows < DH * h + DH),
                           qt_sc[pl.ds(c0, 256), pl.ds(q0, TQ)], 0.0).astype(bf16)

            def chunk(c, mc, h=h, c0=c0, wq=wq):
                m, acc = mc
                k0 = pl.multiple_of(c * sk, sk)
                s = lax.dot_general(kp_sc[pl.ds(k0, sk), pl.ds(c0, 256)].astype(bf16), wq, NN,
                                    preferred_element_type=f32)
                s = (s.astype(bf16).astype(f32) * (4.0 * SCALE_BF16)).astype(bf16).astype(f32)
                m_new = jnp.maximum(m, jnp.max(s, axis=0, keepdims=True))
                p = jnp.exp(s - m_new).astype(bf16)
                pv = lax.dot_general(vt_sc[h, :, pl.ds(k0, sk)], p, NN, preferred_element_type=f32)
                return m_new, acc * jnp.exp(m - m_new) + pv

            init = (jnp.full((1, TQ), -jnp.inf, f32), jnp.zeros((VR, TQ), f32))
            outs.append(normalize(lax.fori_loop(0, S // sk, chunk, init)[1], u))
        put_pair(2 * j, outs[0], outs[1])
        return carry

    lax.cond(flag_sc[0] == 1,
             lambda: lax.fori_loop(0, H // NH, fast_body, 0),
             lambda: lax.fori_loop(0, H // 2, exact_max_body, 0))

    def out_copy(step, n):
        r = n * (TQ // NO)
        return pltpu.make_async_copy(os_sc.at[pl.ds(r, TQ // NO)], o_hbm.at[pl.ds(step * TQ + r, TQ // NO)],
                                     osems.at[n])

    @pl.when(i > 0)
    def _():
        for n in range(NO):
            out_copy(i - 1, n).wait()

    for n in range(NO):
        r, m = n * (TQ // NO), TQ // NO
        if n == 0:
            a = lax.dot_general(wot_sc[...], ot_sc[:, r:r + m].astype(bf16), NN, preferred_element_type=f32).T
        else:
            a = jnp.dot(ot_sc[:, r:r + m].T.astype(bf16), wo_sc[...], preferred_element_type=f32)
        rs = pl.ds(pl.multiple_of(q0 + r, m), m)
        g = jnp.tile(gt_sc[rs, :], (1, NCOL))
        os_sc[r:r + m, :] = (g * a + yb_sc[rs, :]).astype(bf16)
        out_copy(i, n).start()

    @pl.when(i == NQ - 1)
    def _():
        for n in range(NO):
            out_copy(i, n).wait()


@jax.jit
def pallas_gated_mix__softmax_full_mha__dense_activation_squared_relu__prompt_kernel(
    A_x: jax.Array,
    A_wqkv: jax.Array,
    A_wo: jax.Array,
    B_x: jax.Array,
    B_w1: jax.Array,
    B_b1: jax.Array,
    B_w2: jax.Array,
    B_b2: jax.Array,
    gate_w: jax.Array,
):
    del B_x
    vmem = pltpu.VMEM
    scratch = [
        pltpu.SemaphoreType.DMA((NT + len(KV_BLOCKS) + N_LATE,)),
        pltpu.SemaphoreType.DMA((NO,)),
        pltpu.SMEM((1,), i32),
        vmem((TQ, D), bf16),
        vmem((D, D), f32),
        vmem((S, D), bf16), vmem((D, 3 * D), bf16), vmem((D, D), bf16),
        vmem((D, F), bf16), vmem((F, D), bf16),
        vmem((S, D), f32),
        vmem((D, S), f32),
        vmem((H, VR, S), f32),
        vmem((H, S // 4, 128), i32),
        vmem((H, 128, S), i8),
        vmem((H, 1, S), f32),
        vmem((D, TQ), f32),
        vmem((S, D), f32),
        vmem((S, 128), f32),
    ] + [vmem((TK // 2, TQ), i32)] * (2 * NC) + [
        vmem((F,), bf16), vmem((D,), bf16), vmem((D,), bf16),
        vmem((1, D), f32), vmem((1, D + 256), f32),
    ]
    out = pl.pallas_call(
        _kernel,
        grid=(NQ,),
        in_specs=[pl.BlockSpec(memory_space=pl.ANY)] * 8,
        out_specs=pl.BlockSpec(memory_space=pl.ANY),
        out_shape=jax.ShapeDtypeStruct((S, D), bf16),
        scratch_shapes=scratch,
        compiler_params=pltpu.CompilerParams(dimension_semantics=("arbitrary",),
                                             vmem_limit_bytes=100 * 1024 * 1024),
        name="gated_mix_mha_ffn",
    )(A_x.reshape(S, D), A_wqkv, A_wo, B_w1, B_b1, B_w2, B_b2, gate_w)
    return out.reshape(1, S, D)
```

```python
import jax
import jax.numpy as jnp
from jax import lax
import jax.experimental.pallas as pl
import jax.experimental.pallas.tpu as pltpu

S, D, H, DH, F = 2048, 640, 32, 20, 1536
VR = 24
NCOL = D // 128
TQ = 512
TK = 512
NH = 16
TT = 512
KB = 32
NQ, NC, NT = S // TQ, S // TK, S // TT
KV_BLOCKS = ((1280, 1536), (1536, 1920), (640, 768), (768, 1280))
KV_WAIT_AT = (0, 1, 1, 3)
N_LATE = 7
NO = 4

LOG2E = 1.4426950408889634
SCALE_BF16 = 0.2236328125
MAGIC = 12582912.0
QR, KR = 127.0, 254.0
AMAX_LIMIT = 4.0
TINY = 1e-30
f32, bf16, i32, i8 = jnp.float32, jnp.bfloat16, jnp.int32, jnp.int8
NN = (((1,), (0,)), ((), ()))


def _bits(y):
    return lax.bitcast_convert_type(y, i32)


def _zero_after(dep_bits):
    return lax.shift_right_logical(lax.shift_right_logical(dep_bits, 31), 1)


def _after(v, dep):
    if dep is None:
        return v
    return lax.bitcast_convert_type(_bits(v) | _zero_after(_bits(dep)), f32)


def _win(h):
    return DH * h - 4 * (h % 2)


def _kernel(x_hbm, wqkv_hbm, wo_hbm, w1_hbm, b1_hbm, w2_hbm, b2_hbm, gw_hbm, o_hbm,
            sems, osems, flag_sc, os_sc, wot_sc, x_sc, wqkv_sc, wo_sc, w1_sc, w2_sc,
            kp_sc, qt_sc, vt_sc, kh_sc, qh_sc, bq_sc, ot_sc, yb_sc, gt_sc, *rest):
    p_sc = rest[:2 * NC]
    b1_sc, b2_sc, gw_sc, km_sc, ki_sc = rest[2 * NC:]
    i = pl.program_id(0)

    def x_copy(t):
        sl = pl.ds(t * TT, TT)
        return pltpu.make_async_copy(x_hbm.at[sl], x_sc.at[sl], sems.at[t])

    def wcol_copy(n, lo, hi):
        return pltpu.make_async_copy(wqkv_hbm.at[:, lo:hi], wqkv_sc.at[:, lo:hi], sems.at[NT + n])

    nkv = len(KV_BLOCKS)
    kv_copies = [wcol_copy(n, lo, hi) for n, (lo, hi) in enumerate(KV_BLOCKS)]
    late_copies = [wcol_copy(nkv, 0, D)] + [
        pltpu.make_async_copy(src, dst, sems.at[NT + nkv + 1 + n]) for n, (src, dst) in enumerate(
            [(w1_hbm, w1_sc), (w2_hbm, w2_sc), (b1_hbm, b1_sc), (b2_hbm, b2_sc), (gw_hbm, gw_sc),
             (wo_hbm, wo_sc)])]

    def phase_a(t, carry, first=False):
        kmax8, vmax8 = carry
        x_copy(t).wait()
        sl = pl.ds(t * TT if first else pl.multiple_of(t * TT, TT), TT)
        if first:
            parts = []
            for n, (lo, hi) in enumerate(KV_BLOCKS):
                for m in range(nkv):
                    if KV_WAIT_AT[m] == n:
                        kv_copies[m].wait()
                if n == nkv - 1:
                    for tt in range(1, NT):
                        x_copy(tt).start()
                    for cp in late_copies:
                        cp.start()
                parts.append(jnp.dot(x_sc[sl, :], wqkv_sc[:, lo:hi], preferred_element_type=f32))
            vk = jnp.concatenate(parts, axis=1)
            v, k = vk[:, 0:D], vk[:, D:2 * D]
        else:
            xt = x_sc[sl, :]
            v = jnp.dot(xt, wqkv_sc[:, 2 * D:3 * D], preferred_element_type=f32)
            k = jnp.dot(xt, wqkv_sc[:, D:2 * D], preferred_element_type=f32)
        kp_sc[sl, :] = k
        kmax8 = jnp.maximum(kmax8, jnp.max(jnp.abs(k).reshape(TT // 8, 8, D), axis=0))
        vmax8 = jnp.maximum(vmax8, jnp.max(jnp.abs(v).reshape(TT // 8, 8, D), axis=0))
        vT = v.T
        rows = lax.broadcasted_iota(i32, (8, TT), 0)
        for j in range(H // 2):
            mid = vT[40 * j + 16:40 * j + 24]
            vt_sc[2 * j, 0:16, sl] = vT[40 * j:40 * j + 16]
            vt_sc[2 * j, 16:24, sl] = jnp.where(rows < 4, mid, jnp.where(rows == 4, 1.0, 0.0))
            vt_sc[2 * j + 1, 0:8, sl] = jnp.where(rows >= 4, mid, jnp.where(rows == 0, 1.0, 0.0))
            vt_sc[2 * j + 1, 8:24, sl] = vT[40 * j + 24:40 * j + 40]
        return kmax8, vmax8

    def k_split(r0, deps, masks):
        sl = pl.ds(r0, KB)
        sw = pl.ds(pl.multiple_of(r0 // 4, KB // 4), KB // 4)

        def put(lo, n, src, w):
            lo %= 128
            if (lo, n) not in masks:
                lane = lax.broadcasted_iota(i32, (KB // 4, 128), 1)
                masks[lo, n] = ((lane >= lo) & (lane < lo + n) if lo + n <= 128
                                else (lane >= lo) | (lane < lo + n - 128))
            return lax.select(masks[lo, n], src, w)

        limbs = {}
        for c in range(NCOL):
            cs = slice(128 * c, 128 * (c + 1))
            kf = kp_sc[sl, cs] * _after(ki_sc[:, cs], deps[c])
            tk = kf + MAGIC
            ki = tk - MAGIC
            ta = kf * 0.5 + MAGIC
            raw = [_bits(ta), _bits(tk) - _bits(ta), _bits((kf - ki) * 16.0 + MAGIC),
                   _bits(ki * 0.0625 + MAGIC)]
            words = [pltpu.bitcast(r.astype(i8), i32) for r in raw]
            limbs[c] = [pltpu.roll(w, 32 * j, 1) if j else w for j, w in enumerate(words)]
            for h in range(H):
                ch, w0 = divmod(_win(h), 128)
                straddle = w0 + VR > 128
                if ch + int(straddle) != c:
                    continue
                w = limbs[ch][0]
                for j in range(4):
                    if straddle:
                        if j:
                            w = put(w0 + 32 * j, 128 - w0, limbs[ch][j], w)
                        w = put(32 * j, w0 + 32 - 128, limbs[ch + 1][j], w)
                    elif j:
                        w = put(w0 + 32 * j, 32, limbs[ch][j], w)
                kh_sc[h, sw, :] = w

    def q_split(h, qT, kcol, sl, dep):
        rows = lax.broadcasted_iota(i32, (8, TT), 0)
        r0 = _win(h)
        qp = qT[r0:r0 + VR] * jnp.tile(_after(kcol[r0:r0 + VR], dep), (1, TT // 128))
        t3 = [qp[8 * e:8 * e + 8] for e in range(3)]
        if h % 2:
            t3[0] = jnp.where(rows >= 4, t3[0], 0.0)
        else:
            t3[2] = jnp.where(rows < 4, t3[2], 0.0)
        qp = jnp.concatenate(t3, axis=0)
        amax = jnp.maximum(jnp.max(jnp.abs(qp), axis=0, keepdims=True), TINY)
        bq_sc[h, :, sl] = amax * (1.0 / (QR * KR))
        rc = pl.reciprocal(amax, approx=True)
        rc = rc * (2.0 - amax * rc)
        qf = qp * (rc * QR)
        tq = qf + MAGIC
        qi = tq - MAGIC
        raw = [_bits(tq), _bits(tq), _bits(qf * 0.0625 + MAGIC), _bits((qf - qi) * 16.0 + MAGIC)]
        tiles = [jnp.zeros((8, TT), i32)] * 16
        for j, r in enumerate(raw):
            for e in range(3):
                tiles[((r0 % 128) // 8 + 4 * j + e) % 16] = r[8 * e:8 * e + 8]
        qh_sc[h, :, sl] = jnp.concatenate(tiles, axis=0).astype(i8)
        return amax

    def phase_b(t, amax):
        t0 = pl.multiple_of(t * TT, TT)
        sl = pl.ds(t0, TT)
        xt = x_sc[sl, :]
        kcol = jnp.broadcast_to(km_sc[...], (128, D)).T
        q = jnp.dot(xt, wqkv_sc[:, 0:D], preferred_element_type=f32)
        qT = (q * 0.25).T
        qt_sc[:, sl] = qT
        hh = jnp.dot(xt, w1_sc[...], preferred_element_type=f32) + b1_sc[...].astype(f32).reshape(1, F)
        h2 = jnp.maximum(hh, 0.0)
        h2 = (h2 * h2).astype(bf16)
        hb = TT // 2
        bs = [jnp.dot(h2[e * hb:(e + 1) * hb], w2_sc[...], preferred_element_type=f32) for e in range(2)]
        b = jnp.concatenate(bs, axis=0) + b2_sc[...].astype(f32).reshape(1, D)

        pts = [(hh, m, r) for m in range(F // 128) for r in range(8)]
        pts += [(b, m, 4 * e + r) for e in range(2) for m in range(NCOL - e) for r in range(4) for _ in range(2)]

        def point(frac):
            arr, m, r = pts[min(int(frac * len(pts)), len(pts) - 1)]
            return arr[r * (TT // 8):r * (TT // 8) + 1, 128 * m:128 * (m + 1)]

        for h in range(H):
            dep = point(0.3 * (h - H // 2 + 0.5) / (H // 2)) if h >= H // 2 else None
            amax = jnp.maximum(amax, q_split(h, qT, kcol, sl, dep))
        npc, masks = (TT // KB) * NCOL, {}
        for kb in range(TT // KB):
            k_split(pl.multiple_of(t0 + kb * KB, KB),
                    [point(0.3 + 0.7 * (kb * NCOL + c) / npc) for c in range(NCOL)], masks)

        z = jnp.sum(xt.astype(f32) * gw_sc[...].astype(f32).reshape(1, D), axis=-1, keepdims=True)
        g = jax.nn.sigmoid(z)
        yb_sc[sl, :] = (1.0 - g) * b
        gt_sc[sl, :] = jnp.broadcast_to(g, (TT, 128))
        return amax

    def probs(h, c, wq, bq, dst):
        kk = pltpu.bitcast(kh_sc[h, c * TK // 4:(c + 1) * TK // 4, :], i8)
        sc = lax.dot_general(kk, wq, NN, preferred_element_type=i32)
        dst[...] = pltpu.bitcast(jnp.exp2(sc.astype(f32) * bq).astype(bf16), i32)
        return sc[0:8]

    @pl.when(i == 0)
    def _prepare():
        x_copy(0).start()
        for cp in kv_copies:
            cp.start()
        z8 = jnp.zeros((8, D), f32)
        kmax8, vmax8 = lax.fori_loop(1, NT, phase_a, phase_a(0, (z8, z8), first=True))
        kmax = jnp.maximum(jnp.max(kmax8, axis=0, keepdims=True), TINY)
        km_sc[...] = kmax * (4.0 * DH ** -0.5 * LOG2E)
        ki_sc[:, 0:D] = KR / kmax
        vmax = jnp.max(vmax8)
        for cp in late_copies:
            cp.wait()
        amax = lax.fori_loop(0, NT, phase_b, jnp.zeros((1, TT), f32))
        amax = jnp.max(amax, axis=1, keepdims=True)
        pmax = jnp.max(jnp.exp2(jnp.minimum(amax, AMAX_LIMIT) * DH))
        safe = (jnp.max(amax) <= AMAX_LIMIT) & (vmax * pmax <= 2.0 ** 110) & (vmax * 2.0 ** 70 >= pmax)
        flag_sc[0] = safe.astype(i32)
        wot_sc[...] = wo_sc[...].astype(f32).T
        for c in range(NC):
            probs(0, c, qh_sc[0, :, 0:TQ], bq_sc[0, :, 0:TQ], p_sc[c])

    q0 = pl.multiple_of(i * TQ, TQ)

    def normalize(acc, odd):
        return acc * (1.0 / (acc[0:1, :] if odd else acc[DH:DH + 1, :]))

    def put_pair(h_even, oe, oo):
        rows = lax.broadcasted_iota(i32, (8, TQ), 0)
        mid = jnp.where(rows < 4, oe[16:24], oo[0:8])
        ot_sc[pl.ds(pl.multiple_of(DH * h_even, 8), 2 * DH), :] = jnp.concatenate(
            [oe[0:16], mid, oo[8:24]], axis=0)

    def fast_body(jj, carry):
        hb = jj * NH
        zz = pl.multiple_of(lax.shift_right_logical(jj, 16) * 8, 8)
        outs = []
        for u in range(NH):
            if u < NH - 1:
                hn, qn = hb + u + 1, q0
            else:
                last = jj == H // NH - 1
                hn = jnp.where(last, 0, hb + NH)
                qn = pl.multiple_of(jnp.where(last, jnp.minimum(i + 1, NQ - 1) * TQ, q0), TQ)
            wq = qh_sc[hn, :, pl.ds(qn, TQ)]
            bq = bq_sc[hn, :, pl.ds(qn, TQ)]
            acc = None
            for c in range(NC):
                zero = _zero_after(probs(hn, c, wq, bq, p_sc[((u + 1) % 2) * NC + c]))
                pw = p_sc[(u % 2) * NC + c][pl.ds(zz, TK // 2), :]
                pw = jnp.concatenate([piece for e in range(0, TK // 2, 64)
                                      for piece in (pw[e:e + 56], pw[e + 56:e + 64] | zero)], axis=0)
                p = pltpu.bitcast(pw, bf16)
                pv = lax.dot_general(vt_sc[hb + u, :, c * TK:(c + 1) * TK], p, NN,
                                     preferred_element_type=f32)
                acc = pv if acc is None else pv + acc
            outs.append(normalize(acc, u % 2))
            if u % 2:
                put_pair(hb + u - 1, outs[u - 1], outs[u])
        return carry

    def exact_max_body(j, carry):
        sk = 256
        outs = []
        for u in range(2):
            h = 2 * j + u
            c0 = pl.multiple_of(jnp.minimum((DH * h) // 128, NCOL - 2) * 128, 128)
            rows = lax.broadcasted_iota(i32, (256, TQ), 0) + c0
            wq = jnp.where((rows >= DH * h) & (rows < DH * h + DH),
                           qt_sc[pl.ds(c0, 256), pl.ds(q0, TQ)], 0.0).astype(bf16)

            def chunk(c, mc, h=h, c0=c0, wq=wq):
                m, acc = mc
                k0 = pl.multiple_of(c * sk, sk)
                s = lax.dot_general(kp_sc[pl.ds(k0, sk), pl.ds(c0, 256)].astype(bf16), wq, NN,
                                    preferred_element_type=f32)
                s = (s.astype(bf16).astype(f32) * (4.0 * SCALE_BF16)).astype(bf16).astype(f32)
                m_new = jnp.maximum(m, jnp.max(s, axis=0, keepdims=True))
                p = jnp.exp(s - m_new).astype(bf16)
                pv = lax.dot_general(vt_sc[h, :, pl.ds(k0, sk)], p, NN, preferred_element_type=f32)
                return m_new, acc * jnp.exp(m - m_new) + pv

            init = (jnp.full((1, TQ), -jnp.inf, f32), jnp.zeros((VR, TQ), f32))
            outs.append(normalize(lax.fori_loop(0, S // sk, chunk, init)[1], u))
        put_pair(2 * j, outs[0], outs[1])
        return carry

    lax.cond(flag_sc[0] == 1,
             lambda: lax.fori_loop(0, H // NH, fast_body, 0),
             lambda: lax.fori_loop(0, H // 2, exact_max_body, 0))

    def out_copy(step, n):
        r = n * (TQ // NO)
        return pltpu.make_async_copy(os_sc.at[pl.ds(r, TQ // NO)], o_hbm.at[pl.ds(step * TQ + r, TQ // NO)],
                                     osems.at[n])

    @pl.when(i > 0)
    def _():
        for n in range(NO):
            out_copy(i - 1, n).wait()

    for n in range(NO):
        r, m = n * (TQ // NO), TQ // NO
        if n == 0:
            a = lax.dot_general(wot_sc[...], ot_sc[:, r:r + m].astype(bf16), NN, preferred_element_type=f32).T
        else:
            a = jnp.dot(ot_sc[:, r:r + m].T.astype(bf16), wo_sc[...], preferred_element_type=f32)
        rs = pl.ds(pl.multiple_of(q0 + r, m), m)
        g = jnp.tile(gt_sc[rs, :], (1, NCOL))
        os_sc[r:r + m, :] = (g * a + yb_sc[rs, :]).astype(bf16)
        out_copy(i, n).start()

    @pl.when(i == NQ - 1)
    def _():
        for n in range(NO):
            out_copy(i, n).wait()


@jax.jit
def pallas_gated_mix__softmax_full_mha__dense_activation_squared_relu__prompt_kernel(
    A_x: jax.Array,
    A_wqkv: jax.Array,
    A_wo: jax.Array,
    B_x: jax.Array,
    B_w1: jax.Array,
    B_b1: jax.Array,
    B_w2: jax.Array,
    B_b2: jax.Array,
    gate_w: jax.Array,
):
    del B_x
    vmem = pltpu.VMEM
    scratch = [
        pltpu.SemaphoreType.DMA((NT + len(KV_BLOCKS) + N_LATE,)),
        pltpu.SemaphoreType.DMA((NO,)),
        pltpu.SMEM((1,), i32),
        vmem((TQ, D), bf16),
        vmem((D, D), f32),
        vmem((S, D), bf16), vmem((D, 3 * D), bf16), vmem((D, D), bf16),
        vmem((D, F), bf16), vmem((F, D), bf16),
        vmem((S, D), f32),
        vmem((D, S), f32),
        vmem((H, VR, S), f32),
        vmem((H, S // 4, 128), i32),
        vmem((H, 128, S), i8),
        vmem((H, 1, S), f32),
        vmem((D, TQ), f32),
        vmem((S, D), f32),
        vmem((S, 128), f32),
    ] + [vmem((TK // 2, TQ), i32)] * (2 * NC) + [
        vmem((F,), bf16), vmem((D,), bf16), vmem((D,), bf16),
        vmem((1, D), f32), vmem((1, D + 256), f32),
    ]
    out = pl.pallas_call(
        _kernel,
        grid=(NQ,),
        in_specs=[pl.BlockSpec(memory_space=pl.ANY)] * 8,
        out_specs=pl.BlockSpec(memory_space=pl.ANY),
        out_shape=jax.ShapeDtypeStruct((S, D), bf16),
        scratch_shapes=scratch,
        compiler_params=pltpu.CompilerParams(dimension_semantics=("arbitrary",),
                                             vmem_limit_bytes=100 * 1024 * 1024),
        name="gated_mix_mha_ffn",
    )(A_x.reshape(S, D), A_wqkv, A_wo, B_w1, B_b1, B_w2, B_b2, gate_w)
    return out.reshape(1, S, D)
```

```python
import jax
import jax.numpy as jnp
from jax import lax
import jax.experimental.pallas as pl
import jax.experimental.pallas.tpu as pltpu

S, D, H, DH, F = 2048, 640, 32, 20, 1536
VR = 24
NCOL = D // 128
TQ = 512
TK = 512
NH = 16
TT = 512
KB = 32
NQ, NC, NT = S // TQ, S // TK, S // TT
K0, N0 = 256, 1408
N_SEM = NT + 11
NO = 4

LOG2E = 1.4426950408889634
SCALE_BF16 = 0.2236328125
MAGIC = 12582912.0
QR, KR = 127.0, 254.0
AMAX_LIMIT = 4.0
TINY = 1e-30
f32, bf16, i32, i8 = jnp.float32, jnp.bfloat16, jnp.int32, jnp.int8
NN = (((1,), (0,)), ((), ()))


def _bits(y):
    return lax.bitcast_convert_type(y, i32)


def _zero_after(dep_bits):
    return lax.shift_right_logical(lax.shift_right_logical(dep_bits, 31), 1)


def _after(v, dep):
    if dep is None:
        return v
    return lax.bitcast_convert_type(_bits(v) | _zero_after(_bits(dep)), f32)


def _win(h):
    return DH * h - 4 * (h % 2)


def _kernel(x_hbm, wqkv_hbm, wo_hbm, w1_hbm, b1_hbm, w2_hbm, b2_hbm, gw_hbm, o_hbm,
            sems, osems, flag_sc, os_sc, wot_sc, x_sc, wqkv_sc, wo_sc, w1_sc, w2_sc,
            kp_sc, qt_sc, vt_sc, kh_sc, qh_sc, bq_sc, ot_sc, yb_sc, gt_sc, *rest):
    p_sc = rest[:2 * NC]
    b1_sc, b2_sc, gw_sc, km_sc, ki_sc = rest[2 * NC:]
    i = pl.program_id(0)

    def x_copy(t):
        sl = pl.ds(t * TT, TT)
        return pltpu.make_async_copy(x_hbm.at[sl], x_sc.at[sl], sems.at[t])

    def block_copy(src, dst, n, rows, cols):
        r, c = slice(*rows), slice(*cols)
        return pltpu.make_async_copy(src.at[r, c], dst.at[r, c], sems.at[n])

    stage_copies = [
        [block_copy(x_hbm, x_sc, 0, (0, TT), (0, K0)),
         block_copy(wqkv_hbm, wqkv_sc, NT, (0, K0), (N0, 3 * D))],
        [block_copy(x_hbm, x_sc, NT + 1, (0, TT), (K0, D)),
         block_copy(wqkv_hbm, wqkv_sc, NT + 2, (K0, D), (N0, 3 * D))],
        [block_copy(wqkv_hbm, wqkv_sc, NT + 3, (0, D), (D, N0))],
    ]
    late_copies = [block_copy(wqkv_hbm, wqkv_sc, NT + 4, (0, D), (0, D))] + [
        pltpu.make_async_copy(src, dst, sems.at[NT + 5 + n]) for n, (src, dst) in enumerate(
            [(w1_hbm, w1_sc), (w2_hbm, w2_sc), (b1_hbm, b1_sc), (b2_hbm, b2_sc), (gw_hbm, gw_sc),
             (wo_hbm, wo_sc)])]

    def phase_a(t, carry, first=False):
        kmax8, vmax8 = carry
        sl = pl.ds(t * TT if first else pl.multiple_of(t * TT, TT), TT)
        absmax8 = lambda y: jnp.max(jnp.abs(y).reshape(TT // 8, 8, y.shape[1]), axis=0)
        if first:
            def dot2(ks, w):
                return jnp.concatenate(
                    [jnp.dot(x_sc[e * (TT // 2):(e + 1) * (TT // 2), ks], w, preferred_element_type=f32)
                     for e in range(2)], axis=0)

            for cp in stage_copies[0]:
                cp.wait()
            v = dot2(slice(0, K0), wqkv_sc[0:K0, N0:3 * D])
            for cp in stage_copies[1]:
                cp.wait()
            v = dot2(slice(K0, D), wqkv_sc[K0:D, N0:3 * D]) + v
            vtop = absmax8(v)
            for cp in stage_copies[2]:
                cp.wait()
            for tt in range(1, NT):
                x_copy(tt).start()
            for cp in late_copies:
                cp.start()
            vk = dot2(slice(0, D), jnp.concatenate([wqkv_sc[:, 2 * D:N0], wqkv_sc[:, D:2 * D]], axis=1))
            v0, k = vk[:, 0:N0 - 2 * D], vk[:, N0 - 2 * D:]
            v = jnp.concatenate([v0, v], axis=1)
            vtop, ktop = jnp.concatenate([absmax8(v0), vtop], axis=1), absmax8(k)
        else:
            x_copy(t).wait()
            xt = x_sc[sl, :]
            v = jnp.dot(xt, wqkv_sc[:, 2 * D:3 * D], preferred_element_type=f32)
            k = jnp.dot(xt, wqkv_sc[:, D:2 * D], preferred_element_type=f32)
            vtop, ktop = absmax8(v), absmax8(k)
        kp_sc[sl, :] = k
        kmax8, vmax8 = jnp.maximum(kmax8, ktop), jnp.maximum(vmax8, vtop)
        vT = v.T
        rows = lax.broadcasted_iota(i32, (8, TT), 0)
        for j in range(H // 2):
            mid = vT[40 * j + 16:40 * j + 24]
            vt_sc[2 * j, 0:16, sl] = vT[40 * j:40 * j + 16]
            vt_sc[2 * j, 16:24, sl] = jnp.where(rows < 4, mid, jnp.where(rows == 4, 1.0, 0.0))
            vt_sc[2 * j + 1, 0:8, sl] = jnp.where(rows >= 4, mid, jnp.where(rows == 0, 1.0, 0.0))
            vt_sc[2 * j + 1, 8:24, sl] = vT[40 * j + 24:40 * j + 40]
        return kmax8, vmax8

    def k_split(r0, deps, masks):
        sl = pl.ds(r0, KB)
        sw = pl.ds(pl.multiple_of(r0 // 4, KB // 4), KB // 4)

        def put(lo, n, src, w):
            lo %= 128
            if (lo, n) not in masks:
                lane = lax.broadcasted_iota(i32, (KB // 4, 128), 1)
                masks[lo, n] = ((lane >= lo) & (lane < lo + n) if lo + n <= 128
                                else (lane >= lo) | (lane < lo + n - 128))
            return lax.select(masks[lo, n], src, w)

        limbs = {}
        for c in range(NCOL):
            cs = slice(128 * c, 128 * (c + 1))
            kf = kp_sc[sl, cs] * _after(ki_sc[:, cs], deps[c])
            tk = kf + MAGIC
            ki = tk - MAGIC
            ta = kf * 0.5 + MAGIC
            raw = [_bits(ta), _bits(tk) - _bits(ta), _bits((kf - ki) * 16.0 + MAGIC),
                   _bits(ki * 0.0625 + MAGIC)]
            words = [pltpu.bitcast(r.astype(i8), i32) for r in raw]
            limbs[c] = [pltpu.roll(w, 32 * j, 1) if j else w for j, w in enumerate(words)]
            for h in range(H):
                ch, w0 = divmod(_win(h), 128)
                straddle = w0 + VR > 128
                if ch + int(straddle) != c:
                    continue
                w = limbs[ch][0]
                for j in range(4):
                    if straddle:
                        if j:
                            w = put(w0 + 32 * j, 128 - w0, limbs[ch][j], w)
                        w = put(32 * j, w0 + 32 - 128, limbs[ch + 1][j], w)
                    elif j:
                        w = put(w0 + 32 * j, 32, limbs[ch][j], w)
                kh_sc[h, sw, :] = w

    def q_split(h, qT, kcol, sl, dep):
        rows = lax.broadcasted_iota(i32, (8, TT), 0)
        r0 = _win(h)
        qp = qT[r0:r0 + VR] * jnp.tile(_after(kcol[r0:r0 + VR], dep), (1, TT // 128))
        t3 = [qp[8 * e:8 * e + 8] for e in range(3)]
        if h % 2:
            t3[0] = jnp.where(rows >= 4, t3[0], 0.0)
        else:
            t3[2] = jnp.where(rows < 4, t3[2], 0.0)
        qp = jnp.concatenate(t3, axis=0)
        amax = jnp.maximum(jnp.max(jnp.abs(qp), axis=0, keepdims=True), TINY)
        bq_sc[h, :, sl] = amax * (1.0 / (QR * KR))
        rc = pl.reciprocal(amax, approx=True)
        rc = rc * (2.0 - amax * rc)
        qf = qp * (rc * QR)
        tq = qf + MAGIC
        qi = tq - MAGIC
        raw = [_bits(tq), _bits(tq), _bits(qf * 0.0625 + MAGIC), _bits((qf - qi) * 16.0 + MAGIC)]
        tiles = [jnp.zeros((8, TT), i32)] * 16
        for j, r in enumerate(raw):
            for e in range(3):
                tiles[((r0 % 128) // 8 + 4 * j + e) % 16] = r[8 * e:8 * e + 8]
        qh_sc[h, :, sl] = jnp.concatenate(tiles, axis=0).astype(i8)
        return amax

    def phase_b(t, amax):
        t0 = pl.multiple_of(t * TT, TT)
        sl = pl.ds(t0, TT)
        xt = x_sc[sl, :]
        kcol = jnp.broadcast_to(km_sc[...], (128, D)).T
        q = jnp.dot(xt, wqkv_sc[:, 0:D], preferred_element_type=f32)
        qT = (q * 0.25).T
        qt_sc[:, sl] = qT
        hh = jnp.dot(xt, w1_sc[...], preferred_element_type=f32) + b1_sc[...].astype(f32).reshape(1, F)
        h2 = jnp.maximum(hh, 0.0)
        h2 = (h2 * h2).astype(bf16)
        hb = TT // 2
        bs = [jnp.dot(h2[e * hb:(e + 1) * hb], w2_sc[...], preferred_element_type=f32) for e in range(2)]
        b = jnp.concatenate(bs, axis=0) + b2_sc[...].astype(f32).reshape(1, D)

        pts = [(hh, m, r) for m in range(F // 128) for r in range(8)]
        pts += [(b, m, 4 * e + r) for e in range(2) for m in range(NCOL - e) for r in range(4) for _ in range(2)]

        def point(frac):
            arr, m, r = pts[min(int(frac * len(pts)), len(pts) - 1)]
            return arr[r * (TT // 8):r * (TT // 8) + 1, 128 * m:128 * (m + 1)]

        for h in range(H):
            dep = point(0.3 * (h - H // 2 + 0.5) / (H // 2)) if h >= H // 2 else None
            amax = jnp.maximum(amax, q_split(h, qT, kcol, sl, dep))
        npc, masks = (TT // KB) * NCOL, {}
        for kb in range(TT // KB):
            k_split(pl.multiple_of(t0 + kb * KB, KB),
                    [point(0.3 + 0.7 * (kb * NCOL + c) / npc) for c in range(NCOL)], masks)

        z = jnp.sum(xt.astype(f32) * gw_sc[...].astype(f32).reshape(1, D), axis=-1, keepdims=True)
        g = jax.nn.sigmoid(z)
        yb_sc[sl, :] = (1.0 - g) * b
        gt_sc[sl, :] = jnp.broadcast_to(g, (TT, 128))
        return amax

    def probs(h, c, wq, bq, dst):
        kk = pltpu.bitcast(kh_sc[h, c * TK // 4:(c + 1) * TK // 4, :], i8)
        sc = lax.dot_general(kk, wq, NN, preferred_element_type=i32)
        dst[...] = pltpu.bitcast(jnp.exp2(sc.astype(f32) * bq).astype(bf16), i32)
        return sc[0:8]

    @pl.when(i == 0)
    def _prepare():
        for stage in stage_copies:
            for cp in stage:
                cp.start()
        z8 = jnp.zeros((8, D), f32)
        kmax8, vmax8 = lax.fori_loop(1, NT, phase_a, phase_a(0, (z8, z8), first=True))
        kmax = jnp.maximum(jnp.max(kmax8, axis=0, keepdims=True), TINY)
        km_sc[...] = kmax * (4.0 * DH ** -0.5 * LOG2E)
        ki_sc[:, 0:D] = KR / kmax
        for cp in late_copies:
            cp.wait()
        amax = lax.fori_loop(0, NT, phase_b, jnp.zeros((1, TT), f32))
        amax = jnp.max(amax, axis=1, keepdims=True)
        vmax = jnp.max(vmax8)
        pmax = jnp.max(jnp.exp2(jnp.minimum(amax, AMAX_LIMIT) * DH))
        safe = (jnp.max(amax) <= AMAX_LIMIT) & (vmax * pmax <= 2.0 ** 110) & (vmax * 2.0 ** 70 >= pmax)
        flag_sc[0] = safe.astype(i32)
        wot_sc[...] = wo_sc[...].astype(f32).T
        for c in range(NC):
            probs(0, c, qh_sc[0, :, 0:TQ], bq_sc[0, :, 0:TQ], p_sc[c])

    q0 = pl.multiple_of(i * TQ, TQ)

    def normalize(acc, odd):
        return acc * (1.0 / (acc[0:1, :] if odd else acc[DH:DH + 1, :]))

    def put_pair(h_even, oe, oo):
        rows = lax.broadcasted_iota(i32, (8, TQ), 0)
        mid = jnp.where(rows < 4, oe[16:24], oo[0:8])
        ot_sc[pl.ds(pl.multiple_of(DH * h_even, 8), 2 * DH), :] = jnp.concatenate(
            [oe[0:16], mid, oo[8:24]], axis=0)

    def fast_body(jj, carry):
        hb = jj * NH
        zz = pl.multiple_of(lax.shift_right_logical(jj, 16) * 8, 8)
        outs = []
        for u in range(NH):
            if u < NH - 1:
                hn, qn = hb + u + 1, q0
            else:
                last = jj == H // NH - 1
                hn = jnp.where(last, 0, hb + NH)
                qn = pl.multiple_of(jnp.where(last, jnp.minimum(i + 1, NQ - 1) * TQ, q0), TQ)
            wq = qh_sc[hn, :, pl.ds(qn, TQ)]
            bq = bq_sc[hn, :, pl.ds(qn, TQ)]
            acc = None
            for c in range(NC):
                zero = _zero_after(probs(hn, c, wq, bq, p_sc[((u + 1) % 2) * NC + c]))
                pw = p_sc[(u % 2) * NC + c][pl.ds(zz, TK // 2), :]
                pw = jnp.concatenate([piece for e in range(0, TK // 2, 64)
                                      for piece in (pw[e:e + 56], pw[e + 56:e + 64] | zero)], axis=0)
                p = pltpu.bitcast(pw, bf16)
                pv = lax.dot_general(vt_sc[hb + u, :, c * TK:(c + 1) * TK], p, NN,
                                     preferred_element_type=f32)
                acc = pv if acc is None else pv + acc
            outs.append(normalize(acc, u % 2))
            if u % 2:
                put_pair(hb + u - 1, outs[u - 1], outs[u])
        return carry

    def exact_max_body(j, carry):
        sk = 256
        outs = []
        for u in range(2):
            h = 2 * j + u
            c0 = pl.multiple_of(jnp.minimum((DH * h) // 128, NCOL - 2) * 128, 128)
            rows = lax.broadcasted_iota(i32, (256, TQ), 0) + c0
            wq = jnp.where((rows >= DH * h) & (rows < DH * h + DH),
                           qt_sc[pl.ds(c0, 256), pl.ds(q0, TQ)], 0.0).astype(bf16)

            def chunk(c, mc, h=h, c0=c0, wq=wq):
                m, acc = mc
                k0 = pl.multiple_of(c * sk, sk)
                s = lax.dot_general(kp_sc[pl.ds(k0, sk), pl.ds(c0, 256)].astype(bf16), wq, NN,
                                    preferred_element_type=f32)
                s = (s.astype(bf16).astype(f32) * (4.0 * SCALE_BF16)).astype(bf16).astype(f32)
                m_new = jnp.maximum(m, jnp.max(s, axis=0, keepdims=True))
                p = jnp.exp(s - m_new).astype(bf16)
                pv = lax.dot_general(vt_sc[h, :, pl.ds(k0, sk)], p, NN, preferred_element_type=f32)
                return m_new, acc * jnp.exp(m - m_new) + pv

            init = (jnp.full((1, TQ), -jnp.inf, f32), jnp.zeros((VR, TQ), f32))
            outs.append(normalize(lax.fori_loop(0, S // sk, chunk, init)[1], u))
        put_pair(2 * j, outs[0], outs[1])
        return carry

    lax.cond(flag_sc[0] == 1,
             lambda: lax.fori_loop(0, H // NH, fast_body, 0),
             lambda: lax.fori_loop(0, H // 2, exact_max_body, 0))

    def out_copy(step, n):
        r = n * (TQ // NO)
        return pltpu.make_async_copy(os_sc.at[pl.ds(r, TQ // NO)], o_hbm.at[pl.ds(step * TQ + r, TQ // NO)],
                                     osems.at[n])

    @pl.when(i > 0)
    def _():
        for n in range(NO):
            out_copy(i - 1, n).wait()

    for n in range(NO):
        r, m = n * (TQ // NO), TQ // NO
        if n == 0:
            a = lax.dot_general(wot_sc[...], ot_sc[:, r:r + m].astype(bf16), NN, preferred_element_type=f32).T
        else:
            a = jnp.dot(ot_sc[:, r:r + m].T.astype(bf16), wo_sc[...], preferred_element_type=f32)
        rs = pl.ds(pl.multiple_of(q0 + r, m), m)
        g = jnp.tile(gt_sc[rs, :], (1, NCOL))
        os_sc[r:r + m, :] = (g * a + yb_sc[rs, :]).astype(bf16)
        out_copy(i, n).start()

    @pl.when(i == NQ - 1)
    def _():
        for n in range(NO):
            out_copy(i, n).wait()


@jax.jit
def pallas_gated_mix__softmax_full_mha__dense_activation_squared_relu__prompt_kernel(
    A_x: jax.Array,
    A_wqkv: jax.Array,
    A_wo: jax.Array,
    B_x: jax.Array,
    B_w1: jax.Array,
    B_b1: jax.Array,
    B_w2: jax.Array,
    B_b2: jax.Array,
    gate_w: jax.Array,
):
    del B_x
    vmem = pltpu.VMEM
    scratch = [
        pltpu.SemaphoreType.DMA((N_SEM,)),
        pltpu.SemaphoreType.DMA((NO,)),
        pltpu.SMEM((1,), i32),
        vmem((TQ, D), bf16),
        vmem((D, D), f32),
        vmem((S, D), bf16), vmem((D, 3 * D), bf16), vmem((D, D), bf16),
        vmem((D, F), bf16), vmem((F, D), bf16),
        vmem((S, D), f32),
        vmem((D, S), f32),
        vmem((H, VR, S), f32),
        vmem((H, S // 4, 128), i32),
        vmem((H, 128, S), i8),
        vmem((H, 1, S), f32),
        vmem((D, TQ), f32),
        vmem((S, D), f32),
        vmem((S, 128), f32),
    ] + [vmem((TK // 2, TQ), i32)] * (2 * NC) + [
        vmem((F,), bf16), vmem((D,), bf16), vmem((D,), bf16),
        vmem((1, D), f32), vmem((1, D + 256), f32),
    ]
    out = pl.pallas_call(
        _kernel,
        grid=(NQ,),
        in_specs=[pl.BlockSpec(memory_space=pl.ANY)] * 8,
        out_specs=pl.BlockSpec(memory_space=pl.ANY),
        out_shape=jax.ShapeDtypeStruct((S, D), bf16),
        scratch_shapes=scratch,
        compiler_params=pltpu.CompilerParams(dimension_semantics=("arbitrary",),
                                             vmem_limit_bytes=100 * 1024 * 1024),
        name="gated_mix_mha_ffn",
    )(A_x.reshape(S, D), A_wqkv, A_wo, B_w1, B_b1, B_w2, B_b2, gate_w)
    return out.reshape(1, S, D)
```
